```python
import jax
import jax.numpy as jnp

def _softmax(x, axis=-1):
    return jax.nn.softmax(x, axis=axis)

def _gelu(x):
    return jax.nn.gelu(x, approximate=True)

def _silu(x):
    return jax.nn.silu(x)

def _sigmoid(x):
    return jax.nn.sigmoid(x)

def _layernorm(x, axis=-1, eps=1e-05):
    m = jnp.mean(x, axis=axis, keepdims=True)
    v = jnp.var(x, axis=axis, keepdims=True)
    return (x - m) / jnp.sqrt(v + eps)

def _scatter_add(tgt, idx, src, axis=0):
    return tgt.at[idx].add(src)

def _segment_sum(src, seg, n):
    return jax.ops.segment_sum(src, seg, n)

class _Rng:

    def __init__(self, key):
        self._k = key

    def _next(self):
        self._k, sub = jax.random.split(self._k)
        return sub

    def normal(self, shape):
        return jax.random.normal(self._next(), shape, dtype=jnp.bfloat16)

    def randint(self, lo, hi, shape):
        return jax.random.randint(self._next(), shape, lo, hi, dtype=jnp.int32)

    def uniform(self, shape, lo=0.0, hi=1.0):
        return jax.random.uniform(self._next(), shape, jnp.bfloat16, lo, hi)

    def permutation(self, n):
        return jax.random.permutation(self._next(), n)
kernel_name = 'recurrent_scan__memory_aug_recurrent_mem_tr__moe_arch_mod__prompt'

def setup_inputs():
    _rng = _Rng(jax.random.key(int.from_bytes(__import__("os").urandom(4), "little")))
    _w = lambda a: (lambda t: t.astype(jnp.bfloat16) if jnp.issubdtype(t.dtype, jnp.floating) else t)(jnp.asarray(a))

    def _A_setup():
        B, S, Dm = (1, 2048, 640)
        H, Dh = (32, 128)
        M, seg = (8, 32)
        seg = min(seg, S)
        S = S // seg * seg
        return {'x': _w((lambda *s: _rng.normal(s) * 0.05)(B, S, Dm)), 'mem0': _w((lambda *s: _rng.normal(s) * 0.05)(B, M, Dm)), 'Wq': _w((lambda *s: _rng.normal(s) * 0.05)(Dm, H, Dh) * Dm ** (-0.5)), 'Wk': _w((lambda *s: _rng.normal(s) * 0.05)(Dm, H, Dh) * Dm ** (-0.5)), 'Wv': _w((lambda *s: _rng.normal(s) * 0.05)(Dm, H, Dh) * Dm ** (-0.5)), 'Wo': _w((lambda *s: _rng.normal(s) * 0.05)(H, Dh, Dm) * (H * Dh) ** (-0.5)), 'seg_len': seg}
    _A_in = _A_setup()

    def _B_setup():
        B, S, D, F, C = (1, 2048, 640, 1728, 8)
        return {'x': _w((lambda *s: _rng.normal(s) * 0.05)(B, S, D)), 'w_r': _w((lambda *s: _rng.normal(s) * 0.05)(D)), 'w_gate': _w((lambda *s: _rng.normal(s) * 0.05)(D, F)), 'w_up': _w((lambda *s: _rng.normal(s) * 0.05)(D, F)), 'w_down': _w((lambda *s: _rng.normal(s) * 0.05)(F, D))}
    _B_in = _B_setup()
    return {'A_x': _A_in['x'], 'A_mem0': _A_in['mem0'], 'A_Wq': _A_in['Wq'], 'A_Wk': _A_in['Wk'], 'A_Wv': _A_in['Wv'], 'A_Wo': _A_in['Wo'], 'A_seg_len': _A_in['seg_len'], 'B_x': _B_in['x'], 'B_w_r': _B_in['w_r'], 'B_w_gate': _B_in['w_gate'], 'B_w_up': _B_in['w_up'], 'B_w_down': _B_in['w_down']}

def reference(A_x, A_mem0, A_Wq, A_Wk, A_Wv, A_Wo, A_seg_len, B_x, B_w_r, B_w_gate, B_w_up, B_w_down):

    def _A_ref(x, mem0, Wq, Wk, Wv, Wo, seg_len):
        B, S, Dm = x.shape
        H, Dh = (Wq.shape[1], Wq.shape[2])
        M = mem0.shape[1]
        scale = Dh ** (-0.5)
        n_seg = S // seg_len
        L = M + seg_len
        idx = jnp.arange(L)
        mask = (idx[:, None] < M) | (idx[:, None] >= idx[None, :])
        mem = mem0
        outs = []
        for s in range(n_seg):
            xs = x[:, s * seg_len:(s + 1) * seg_len, :].copy()
            h = jnp.concatenate([mem, xs], axis=1)
            q = jnp.einsum('btd,dhe->bhte', h, Wq)
            k = jnp.einsum('btd,dhe->bhte', h, Wk)
            v = jnp.einsum('btd,dhe->bhte', h, Wv)
            scores = jnp.einsum('bhqe,bhke->bhqk', q, k) * scale
            scores = jnp.where(mask[None, None], scores, -1000000000.0)
            p = _softmax(scores, axis=-1)
            o = jnp.einsum('bhqk,bhke->bhqe', p, v)
            o = jnp.einsum('bhte,hed->btd', o, Wo)
            mem = o[:, :M, :].copy()
            outs.append(o[:, M:, :])
        return jnp.concatenate(outs, axis=1)

    def _B_ref(x, w_r, w_gate, w_up, w_down):
        B, S, D = x.shape
        C = 8
        r = x @ w_r
        idx = jnp.argsort(-r, axis=-1)[:, :C]
        idx_e = jnp.repeat(idx.reshape(B, C, 1), D, axis=2)
        x_sel = jnp.take_along_axis(x, idx_e, axis=1)
        g = _silu(x_sel @ w_gate)
        u = x_sel @ w_up
        y = g * u @ w_down
        r_sel = _sigmoid(jnp.take_along_axis(r, idx, axis=1))
        y = y * r_sel.reshape(B, C, 1)
        b_off = (jnp.arange(B) * S).reshape(B, 1)
        flat_idx = (idx + b_off).reshape(B * C)
        zero = (x * 0.0).reshape(B * S, D)
        upd = _scatter_add(zero, flat_idx, y.reshape(B * C, D), axis=0)
        return x + upd.reshape(B, S, D)
    x = A_x
    xn = _layernorm(x, axis=-1)
    s = _A_ref(xn, A_mem0, A_Wq, A_Wk, A_Wv, A_Wo, A_seg_len)
    g = _silu(_B_ref(xn, B_w_r, B_w_gate, B_w_up, B_w_down))
    return x + s * g
```

```python
import functools

import jax
import jax.numpy as jnp
from jax import lax
import jax.experimental.pallas as pl
import jax.experimental.pallas.tpu as pltpu

bf16 = jnp.bfloat16
f32 = jnp.float32
u32 = jnp.uint32

S, D, H, E = 2048, 640, 32, 128
M, SEG = 8, 32
NSEG = S // SEG
NP = H // 2
F, C = 1728, 8
KT = D // 128
PITCH = 328
EPS_BF16 = 1.0013580322265625e-05
NT = (((1,), (1,)), ((), ()))

DQK, DPV, SPLIT = 1, 3, 13


def _rb(v):
    return v.astype(bf16).astype(f32)


def _masks():
    r = lax.broadcasted_iota(jnp.int32, (80, 80), 0)
    c = lax.broadcasted_iota(jnp.int32, (80, 80), 1)

    def head(i):
        return jnp.where(i < 64, i >> 5, (i - 64) >> 3)

    def pos(i):
        j = i & 31
        return jnp.where(i < 64, jnp.where(j < 8, j, j + 8), 8 + (i & 7))

    same = head(r) == head(c)
    pr, pc = pos(r), pos(c)
    keep = same & ((pr < M) | (pr >= pc))
    fill = jnp.where(same, -1000000000.0, -jnp.inf).astype(f32)
    return keep, fill


def _kernel(x_hbm, mem0_ref, wq_hbm, wk_hbm, wv_hbm, wo_hbm, wr_ref, wg_hbm, wu_hbm, wd_hbm,
            out_hbm,
            xbuf, xn32, xb32, xnb, r_ref, sel_ref, wraw, wqkv, wo_raw, wo32, qkvb, ob,
            wg, wu, wd, obuf, accs, sems):
    w_hbm = (wq_hbm, wk_hbm, wv_hbm)

    cp_x = pltpu.make_async_copy(x_hbm, xbuf, sems.at[0])
    cp_w = [pltpu.make_async_copy(w_hbm[c // 2].at[:, pl.ds(16 * (c % 2), 16), :], wraw.at[c],
                                  sems.at[1 + c]) for c in range(6)]
    cp_wo = pltpu.make_async_copy(wo_hbm, wo_raw, sems.at[7])
    cp_wg = pltpu.make_async_copy(wg_hbm, wg, sems.at[8])
    cp_wu = pltpu.make_async_copy(wu_hbm, wu, sems.at[9])
    cp_wd = pltpu.make_async_copy(wd_hbm, wd, sems.at[10])
    later = cp_w[2:] + [cp_wo, cp_wg, cp_wu, cp_wd]

    cp_x.start()
    cp_w[0].start()
    cp_x.wait()
    cp_w[1].start()

    wr16 = jnp.broadcast_to(wr_ref[...].astype(f32).reshape(1, D), (16, D)).astype(bf16)

    def ln_body(i, carry):
        r0 = pl.multiple_of(i * 128, 128)
        x = xbuf[pl.ds(r0, 128), :].astype(f32)
        mu = jnp.mean(x, axis=-1, keepdims=True)
        xc = x - mu
        var = jnp.mean(xc * xc, axis=-1, keepdims=True)
        den = _rb(jnp.sqrt(_rb(_rb(var) + EPS_BF16)))
        xn = (_rb(x - _rb(mu)) / den).astype(bf16)
        xf = xn.astype(f32)
        xn32[pl.ds(r0, 128), :] = xf
        xb32[pl.ds(r0, 128), :] = xf
        xB = jnp.concatenate([xf[32 * j:32 * j + 8] for j in range(4)], axis=0).astype(bf16)
        xnb[pl.ds(pl.multiple_of(i * 16, 16), 16), :] = pltpu.bitcast(xB, u32)
        rr = lax.dot_general(wr16, xn, NT, preferred_element_type=f32)
        r_ref[pl.ds(i, 1), :] = rr[0:1]
        return carry

    lax.fori_loop(0, S // 128, ln_body, 0)

    def relayout(c, i):
        t, g = c // 2, c % 2
        for j in range(8):
            dd = i * 8 + j
            a = pltpu.bitcast(wraw[c, 2 * dd], u32)
            b = pltpu.bitcast(wraw[c, 2 * dd + 1], u32)
            lo = (a & jnp.uint32(0xFFFF)) | (b << 16)
            hi = (a >> 16) | (b & jnp.uint32(0xFFFF0000))
            base = g * 8 * PITCH + dd
            wqkv[t, 0, pl.ds(base, 8, stride=PITCH), :] = lo
            wqkv[t, 1, pl.ds(base, 8, stride=PITCH), :] = hi

    def wtile(t, par, hp):
        start = hp * PITCH
        if not isinstance(hp, int):
            start = pl.multiple_of(start, 8)
        return pltpu.bitcast(wqkv[t, par, pl.ds(start, D // 2), :], bf16)

    for c in range(6):
        cp_w[c].wait()
        for cp in later[2 * c:2 * c + 2]:
            cp.start()

        def rl_body(i, carry, c=c):
            relayout(c, i)
            return carry

        lax.fori_loop(0, 40, rl_body, 0)

        def pp_body(p, carry, c=c):
            t, hp = c // 2, (c % 2) * 8 + p
            w0, w1 = wtile(t, 0, hp), wtile(t, 1, hp)
            for mb in range(4):
                lhs = pltpu.bitcast(xnb[mb * 64:(mb + 1) * 64, :], bf16)
                y0 = jnp.dot(lhs, w0, preferred_element_type=f32).reshape(16, 8, E)
                y1 = jnp.dot(lhs, w1, preferred_element_type=f32).reshape(16, 8, E)
                y = jnp.concatenate([y0, y1], axis=1).astype(bf16)
                qkvb[t, hp, mb * 16:(mb + 1) * 16] = pltpu.bitcast(y, u32)
            return carry

        lax.fori_loop(0, 8, pp_body, 0)

    cp_wo.wait()

    def wo_body(i, carry):
        r0 = pl.multiple_of(i * 128, 128)
        w = pltpu.bitcast(wo_raw[pl.ds(r0, 128), :], u32)
        for n in range(KT):
            wo32[n, pl.ds(pl.multiple_of(i * 64, 64), 64), :] = w[:, n * 128:(n + 1) * 128]
        return carry

    lax.fori_loop(0, H, wo_body, 0)

    r = _rb(r_ref[...])
    tok = (lax.broadcasted_iota(jnp.int32, (16, 128), 0) * 128
           + lax.broadcasted_iota(jnp.int32, (16, 128), 1)).astype(f32)
    row16 = lax.broadcasted_iota(jnp.int32, (16, 1), 0)
    sel_ref[...] = jnp.zeros(sel_ref.shape, f32)
    gate = jnp.zeros((16, 1), f32)
    taken = jnp.zeros((16, 128), jnp.bool_)
    idxs = []
    for j in range(C):
        best = jnp.max(jnp.where(taken, -jnp.inf, r), keepdims=True)
        hit = jnp.logical_and(r == best, jnp.logical_not(taken))
        pick = jnp.min(jnp.where(hit, tok, float(S - 1)), keepdims=True)
        taken = jnp.logical_or(taken, tok == pick)
        gate = jnp.where(row16 == j, best, gate)
        idx = jnp.clip(pick[0, 0].astype(jnp.int32), 0, S - 1)
        idxs.append(idx)
        sel_ref[j:j + 1, :] = xn32[pl.ds(idx, 1), :]
    cp_wg.wait()
    cp_wu.wait()
    cp_wd.wait()
    xs = sel_ref[...]
    xsb = xs.astype(bf16)
    hg = lax.dot_general(xsb, wg[...], NT, preferred_element_type=f32)
    hu = lax.dot_general(xsb, wu[...], NT, preferred_element_type=f32)
    hh = (hg * jax.nn.sigmoid(hg) * hu).astype(bf16)
    y = jnp.dot(hh, wd[...], preferred_element_type=f32)
    xs = xs + y * jax.nn.sigmoid(gate)
    for j in range(C):
        xb32[pl.ds(idxs[j], 1), :] = xs[j:j + 1]

    def finish(rows, s_val):
        b = xb32[rows, :]
        x = xbuf[rows, :].astype(f32)
        obuf[rows, :] = (x + s_val * (b * jax.nn.sigmoid(b))).astype(bf16)

    keep, fill = _masks()
    scale = E ** -0.5

    def step(s, mem):
        r0 = pl.multiple_of(s * SEG, SEG)
        rows_a = pl.ds(r0 + 8, 24)
        lhs = jnp.concatenate([mem, xn32[rows_a, :]], axis=0).astype(bf16)
        st = {}

        def qkv(hp):
            res = []
            for t in range(3):
                y0 = jnp.dot(lhs, wtile(t, 0, hp), preferred_element_type=f32).astype(bf16)
                y1 = jnp.dot(lhs, wtile(t, 1, hp), preferred_element_type=f32).astype(bf16)
                yb = pltpu.bitcast(qkvb[t, hp, s], bf16)
                res.append(jnp.concatenate([y0, y1, yb], axis=0))
            st['qkv', hp] = res

        def qk(hp):
            q, k, _ = st['qkv', hp]
            sc = lax.dot_general(q, k, NT, preferred_element_type=f32) * scale
            sc = jnp.where(keep, sc, fill)
            p = jnp.exp(sc - jnp.max(sc, axis=-1, keepdims=True))
            l = jnp.sum(p, axis=-1, keepdims=True)
            st['p', hp] = (p * pl.reciprocal(l, approx=True)).astype(bf16)

        def pv(hp):
            o = jnp.dot(st['p', hp], st['qkv', hp][2], preferred_element_type=f32)
            st['o', 2 * hp] = o[0:32].astype(bf16)
            st['o', 2 * hp + 1] = o[32:64].astype(bf16)
            rb = pl.ds(pl.multiple_of(s * 8, 8), 8)
            ob[2 * hp, rb, :] = o[64:72]
            ob[2 * hp + 1, rb, :] = o[72:80]

        def oproj(n, h0, h1):
            a = jnp.concatenate([st['o', h] for h in range(h0, h1)], axis=1)
            w = pltpu.bitcast(wo32[n, h0 * 64:h1 * 64, :], bf16)
            return jnp.dot(a, w, preferred_element_type=f32)

        for t in range(NP + KT):
            if t < NP:
                qkv(t)
            else:
                accs[t - NP] = oproj(t - NP, 0, 2 * SPLIT)
            if 0 <= t - DQK < NP:
                qk(t - DQK)
            if 0 <= t - DPV < NP:
                pv(t - DPV)
        acc = jnp.concatenate([accs[n] + oproj(n, 2 * SPLIT, H) for n in range(KT)], axis=1)
        finish(rows_a, acc[8:32])
        return _rb(acc[0:8])

    lax.fori_loop(0, NSEG, step, mem0_ref[...].astype(f32))

    def out_copy(mb):
        rows = pl.ds(mb * 512, 512)
        return pltpu.make_async_copy(obuf.at[rows, :], out_hbm.at[rows, :], sems.at[11 + mb])

    for mb in range(4):
        a = jnp.concatenate([ob[h, mb * 128:(mb + 1) * 128, :].astype(bf16) for h in range(H)],
                            axis=1)
        res = jnp.concatenate(
            [jnp.dot(a, pltpu.bitcast(wo32[n], bf16), preferred_element_type=f32)
             for n in range(KT)], axis=1)
        for j in range(16):
            finish(pl.ds((mb * 16 + j) * SEG, 8), res[8 * j:8 * j + 8])
        out_copy(mb).start()
    for mb in range(4):
        out_copy(mb).wait()


@functools.partial(jax.jit, static_argnames=("A_seg_len",))
def pallas_recurrent_scan__memory_aug_recurrent_mem_tr__moe_arch_mod__prompt_kernel(
    A_x: jax.Array,
    A_mem0: jax.Array,
    A_Wq: jax.Array,
    A_Wk: jax.Array,
    A_Wv: jax.Array,
    A_Wo: jax.Array,
    A_seg_len,
    B_x: jax.Array,
    B_w_r: jax.Array,
    B_w_gate: jax.Array,
    B_w_up: jax.Array,
    B_w_down: jax.Array,
):
    del B_x
    assert A_seg_len == SEG
    assert A_x.shape == (1, S, D) and A_Wq.shape == (D, H, E) and B_w_gate.shape == (D, F)
    hbm = pl.BlockSpec(memory_space=pl.ANY)
    vmem = pl.BlockSpec(memory_space=pltpu.VMEM)
    out = pl.pallas_call(
        _kernel,
        out_shape=jax.ShapeDtypeStruct((S, D), bf16),
        in_specs=[hbm, vmem, hbm, hbm, hbm, hbm, vmem, hbm, hbm, hbm],
        out_specs=hbm,
        scratch_shapes=[
            pltpu.VMEM((S, D), bf16),
            pltpu.VMEM((S, D), f32),
            pltpu.VMEM((S, D), f32),
            pltpu.VMEM((NSEG * 4, D), u32),
            pltpu.VMEM((16, 128), f32),
            pltpu.VMEM((16, D), f32),
            pltpu.VMEM((6, D, 16, E), bf16),
            pltpu.VMEM((3, 2, NP * PITCH, E), u32),
            pltpu.VMEM((H * E, D), bf16),
            pltpu.VMEM((KT, H * E // 2, 128), u32),
            pltpu.VMEM((3, NP, NSEG, 8, E), u32),
            pltpu.VMEM((H, NSEG * 8, E), f32),
            pltpu.VMEM((F, D), bf16),
            pltpu.VMEM((F, D), bf16),
            pltpu.VMEM((F, D), bf16),
            pltpu.VMEM((S, D), bf16),
            pltpu.VMEM((KT, 32, 128), f32),
            pltpu.SemaphoreType.DMA((15,)),
        ],
        compiler_params=pltpu.CompilerParams(vmem_limit_bytes=120 * 1024 * 1024),
    )(A_x.reshape(S, D), A_mem0.reshape(M, D), A_Wq, A_Wk, A_Wv, A_Wo.reshape(H * E, D),
      B_w_r, B_w_gate.T, B_w_up.T, B_w_down)
    return out.reshape(1, S, D)
```

```python
import functools

import jax
import jax.numpy as jnp
from jax import lax
import jax.experimental.pallas as pl
import jax.experimental.pallas.tpu as pltpu

bf16 = jnp.bfloat16
f32 = jnp.float32
u32 = jnp.uint32

S, D, H, E = 2048, 640, 32, 128
M, SEG = 8, 32
NSEG = S // SEG
NP = H // 2
F, C = 1728, 8
KT = D // 128
NCH = 12
PITCH = 328
EPS_BF16 = 1.0013580322265625e-05
NT = (((1,), (1,)), ((), ()))

DQK, DPV, SPLIT = 1, 3, 13
import os
LNB, LNA = 8, int(os.environ.get('LNA', 2))
LNA_LAG = tuple(int(c) for c in os.environ.get('LAG', '0123'))
FILL_PLAN = ((), (0, 1), (2, 3), (4,))


def _rb(v):
    return v.astype(bf16).astype(f32)


def _masks():
    r = lax.broadcasted_iota(jnp.int32, (80, 80), 0)
    c = lax.broadcasted_iota(jnp.int32, (80, 80), 1)

    def head(i):
        return jnp.where(i < 64, i >> 5, (i - 64) >> 3)

    def pos(i):
        j = i & 31
        return jnp.where(i < 64, jnp.where(j < 8, j, j + 8), 8 + (i & 7))

    same = head(r) == head(c)
    pr, pc = pos(r), pos(c)
    keep = same & ((pr < M) | (pr >= pc))
    fill = jnp.where(same, -1000000000.0, -jnp.inf).astype(f32)
    return keep, fill


def _interleave(units, side):
    done = 0
    for i, unit in enumerate(units):
        unit()
        want = (len(side) * (i + 1)) // len(units)
        for task in side[done:want]:
            task()
        done = want


def _kernel(x_hbm, mem0_ref, wq_hbm, wk_hbm, wv_hbm, wo_hbm, wr_ref, wg_hbm, wu_hbm, wd_hbm,
            out_hbm,
            xbuf, xa32, xb32, xnb, sel_ref, hh_ref, wraw, wo, qkvb, ob,
            wg, wu, wd, obuf, accs, accb, sems, osems, *wqkv):
    w_hbm = (wq_hbm, wk_hbm, wv_hbm)

    cp_xb = pltpu.make_async_copy(x_hbm.at[:, pl.ds(0, 8), :], xbuf.at[:, pl.ds(0, 8), :],
                                  sems.at[0])
    cp_xa = pltpu.make_async_copy(x_hbm.at[:, pl.ds(8, 24), :], xbuf.at[:, pl.ds(8, 24), :],
                                  sems.at[1])
    cp_w = [pltpu.make_async_copy(w_hbm[c // 4].at[:, pl.ds(8 * (c % 4), 8), :], wraw.at[c],
                                  sems.at[2 + c]) for c in range(NCH)]
    cp_ffn = [pltpu.make_async_copy(src, dst, sems.at[14 + i])
              for i, (src, dst) in enumerate(((wg_hbm, wg), (wu_hbm, wu), (wd_hbm, wd)))]
    cp_wo = [pltpu.make_async_copy(wo_hbm.at[:, pl.ds(128 * n, 128)], wo.at[n], sems.at[17 + n])
             for n in range(KT)]
    for cp in [cp_xb] + cp_w[:7] + [cp_xa] + cp_w[7:] + cp_ffn + cp_wo:
        cp.start()

    wr = wr_ref[...].astype(f32).reshape(1, D)
    lane = lax.broadcasted_iota(jnp.int32, (8, 128), 1)
    scores = [jnp.zeros((8, 128), f32), jnp.zeros((8, 128), f32)]

    def layernorm(n, load, store, groups, lag):
        st = {}

        def mean(i):
            st['mu', i] = jnp.mean(load(i), axis=-1, keepdims=True)

        def var(i):
            xc = load(i) - st['mu', i]
            st['var', i] = jnp.mean(xc * xc, axis=-1, keepdims=True)

        def norm(i):
            den = _rb(jnp.sqrt(_rb(_rb(st['var', i]) + EPS_BF16)))
            xn = _rb(_rb(load(i) - _rb(st['mu', i])) * (1.0 / den))
            store(i, xn)
            st['r', i] = jnp.sum(xn * wr, axis=-1, keepdims=True)

        def score(i):
            for k, g in enumerate(groups(i)):
                scores[g // 128] = jnp.where(lane == g % 128, st['r', i][8 * k:8 * k + 8],
                                             scores[g // 128])

        def stage(t):
            for d, fn in zip(lag, (mean, var, norm, score)):
                if 0 <= t - d < n:
                    fn(t - d)

        return [functools.partial(stage, t) for t in range(n + lag[-1])]

    def store_b(i, xn):
        for k in range(LNB):
            xb32[(LNB * i + k) * SEG:(LNB * i + k) * SEG + 8, :] = xn[8 * k:8 * k + 8]
        xnb[4 * LNB * i:4 * LNB * (i + 1), :] = pltpu.bitcast(xn.astype(bf16), u32)

    def store_a(i, xn):
        for k in range(LNA):
            sg = LNA * i + k
            xb32[sg * SEG + 8:(sg + 1) * SEG, :] = xn[24 * k:24 * k + 24]
            xa32[sg] = xn[24 * k:24 * k + 24]

    ln_b = layernorm(
        NSEG // LNB,
        lambda i: xbuf[LNB * i:LNB * (i + 1), 0:8, :].astype(f32).reshape(8 * LNB, D),
        store_b, lambda i: [4 * (LNB * i + k) for k in range(LNB)], (0, 1, 2, 3))
    ln_a = layernorm(
        NSEG // LNA,
        lambda i: xbuf[LNA * i:LNA * (i + 1), 8:32, :].astype(f32).reshape(24 * LNA, D),
        store_a, lambda i: [4 * (LNA * i + k) + j for k in range(LNA) for j in (1, 2, 3)],
        LNA_LAG)

    def relayout(c, i):
        for dd in range(16 * i, 16 * i + 16):
            a = pltpu.bitcast(wraw[c, 2 * dd], u32)
            b = pltpu.bitcast(wraw[c, 2 * dd + 1], u32)
            rows = pl.ds(dd, 4, stride=PITCH)
            wqkv[c][0, rows, :] = (a & jnp.uint32(0xFFFF)) | (b << 16)
            wqkv[c][1, rows, :] = (a >> 16) | (b & jnp.uint32(0xFFFF0000))

    def wtile(t, par, hp):
        start = (hp % 4) * PITCH
        w = wqkv[4 * t + hp // 4][par, start:start + D // 2, :]
        return pltpu.bitcast(w, bf16)

    def prepass(c, p, mb):
        t, hp = c // 4, (c % 4) * 4 + p
        lhs = pltpu.bitcast(xnb[mb * 64:(mb + 1) * 64, :], bf16)
        y0 = jnp.dot(lhs, wtile(t, 0, hp), preferred_element_type=f32).reshape(16, 8, E)
        y1 = jnp.dot(lhs, wtile(t, 1, hp), preferred_element_type=f32).reshape(16, 8, E)
        y = jnp.concatenate([y0, y1], axis=1).astype(bf16)
        qkvb[t, hp, mb * 16:(mb + 1) * 16] = pltpu.bitcast(y, u32)

    route = {}

    def top_c():
        r = _rb(jnp.concatenate(scores, axis=1))
        tok = (lax.broadcasted_iota(jnp.int32, (8, 256), 1) * 8
               + lax.broadcasted_iota(jnp.int32, (8, 256), 0)).astype(f32)
        row16 = lax.broadcasted_iota(jnp.int32, (16, 1), 0)
        sel_ref[8:16, :] = jnp.zeros((8, D), f32)
        gate = jnp.zeros((16, 1), f32)
        taken = jnp.zeros((8, 256), jnp.bool_)
        idxs = []
        for j in range(C):
            best = jnp.max(jnp.where(taken, -jnp.inf, r), keepdims=True)
            hit = jnp.logical_and(r == best, jnp.logical_not(taken))
            pick = jnp.min(jnp.where(hit, tok, float(S - 1)), keepdims=True)
            taken = jnp.logical_or(taken, tok == pick)
            gate = jnp.where(row16 == j, best, gate)
            idx = jnp.clip(pick[0, 0].astype(jnp.int32), 0, S - 1)
            idxs.append(idx)
            sel_ref[j:j + 1, :] = xb32[pl.ds(idx, 1), :]
        route['idx'] = idxs
        route['gate'] = jax.nn.sigmoid(gate)

    def ffn_up(n):
        cols = slice(128 * n, min(128 * (n + 1), F))
        xsb = sel_ref[...].astype(bf16)
        hg = lax.dot_general(xsb, wg[cols, :], NT, preferred_element_type=f32)
        hu = lax.dot_general(xsb, wu[cols, :], NT, preferred_element_type=f32)
        hh_ref[:, cols] = hg * jax.nn.sigmoid(hg) * hu

    def ffn_down(n):
        cols = slice(128 * n, 128 * (n + 1))
        y = jnp.dot(hh_ref[...].astype(bf16), wd[:, cols], preferred_element_type=f32)
        sel_ref[:, cols] = sel_ref[:, cols] + y * route['gate']

    def ffn_scatter():
        for j in range(C):
            xb32[pl.ds(route['idx'][j], 1), :] = sel_ref[j:j + 1, :]

    P = functools.partial
    pp = lambda c, ps=range(4): [P(prepass, c, p, mb) for p in ps for mb in range(4)]
    rl = lambda c: [P(relayout, c, i) for i in range(20)]

    def block(name, waits, units, side):
        with jax.named_scope("wait_" + name):
            for cp in waits:
                cp.wait()
        with jax.named_scope("blk_" + name):
            _interleave(units, side)

    block("lnb", [cp_xb], ln_b, [])
    block("0", cp_w[0:1], rl(0) + pp(0, (0, 1)), [])
    block("1", cp_w[1:2], pp(0, (2, 3)), rl(1))
    block("2", cp_w[2:3], pp(1), rl(2))
    block("3", cp_w[3:5], pp(2), rl(3) + rl(4))
    block("4", cp_w[5:7], pp(3) + pp(4), rl(5) + rl(6))
    block("5", [cp_xa] + cp_w[7:9], pp(5) + pp(6), ln_a + rl(7) + rl(8))
    block("6", cp_w[9:12], pp(7) + pp(8), [top_c] + rl(9) + rl(10) + rl(11))
    block("7", cp_ffn, pp(9) + pp(10) + pp(11),
          [P(ffn_up, n) for n in range(14)] + [P(ffn_down, n) for n in range(KT)] + [ffn_scatter])
    block("wo", cp_wo, [], [])

    def finish(s, lo, n, s_val):
        r0 = s * SEG if isinstance(s, int) else pl.multiple_of(s * SEG, SEG)
        b = xb32[pl.ds(r0 + lo, n), :]
        x = xbuf[s, lo:lo + n, :].astype(f32)
        obuf[s, lo:lo + n, :] = (x + s_val * (b * jax.nn.sigmoid(b))).astype(bf16)

    keep, fill = _masks()
    scale = E ** -0.5

    def step(s, mem):
        lhs = jnp.concatenate([mem, xa32[s]], axis=0).astype(bf16)
        st = {}

        def qkv(hp):
            res = []
            for t in range(3):
                y0 = jnp.dot(lhs, wtile(t, 0, hp), preferred_element_type=f32).astype(bf16)
                y1 = jnp.dot(lhs, wtile(t, 1, hp), preferred_element_type=f32).astype(bf16)
                yb = pltpu.bitcast(qkvb[t, hp, s], bf16)
                res.append(jnp.concatenate([y0, y1, yb], axis=0))
            st['qkv', hp] = res

        def qk(hp):
            q, k, _ = st['qkv', hp]
            sc = lax.dot_general(q, k, NT, preferred_element_type=f32) * scale
            sc = jnp.where(keep, sc, fill)
            p = jnp.exp(sc - jnp.max(sc, axis=-1, keepdims=True))
            l = jnp.sum(p, axis=-1, keepdims=True)
            st['p', hp] = (p * pl.reciprocal(l, approx=True)).astype(bf16)

        def pv(hp):
            o = jnp.dot(st['p', hp], st['qkv', hp][2], preferred_element_type=f32)
            st['o', 2 * hp] = o[0:32].astype(bf16)
            st['o', 2 * hp + 1] = o[32:64].astype(bf16)
            rb = pl.ds(s * 8 if isinstance(s, int) else pl.multiple_of(s * 8, 8), 8)
            ob[2 * hp, rb, :] = o[64:72]
            ob[2 * hp + 1, rb, :] = o[72:80]

        def oproj(n, h0, h1):
            a = jnp.concatenate([st['o', h] for h in range(h0, h1)], axis=1)
            w = wo[n, h0 * 128:h1 * 128, :]
            return jnp.dot(a, w, preferred_element_type=f32)

        for t in range(NP + KT):
            if t < NP:
                qkv(t)
            else:
                accs[t - NP] = oproj(t - NP, 0, 2 * SPLIT)
            if 0 <= t - DQK < NP:
                qk(t - DQK)
            if 0 <= t - DPV < NP:
                pv(t - DPV)
        acc = jnp.concatenate([accs[n] + oproj(n, 2 * SPLIT, H) for n in range(KT)], axis=1)
        finish(s, 8, 24, acc[8:32])
        return _rb(acc[0:8])

    def oproj_b(g, n):
        rows = pl.ds(g * 32 if isinstance(g, int) else pl.multiple_of(g * 32, 32), 32)
        a = jnp.concatenate([ob[h, rows, :].astype(bf16) for h in range(H)], axis=1)
        accb[n] = jnp.dot(a, wo[n], preferred_element_type=f32)

    def finish_b(g):
        res = jnp.concatenate([accb[n] for n in range(KT)], axis=1)
        for j in range(4):
            finish(g * 4 + j, 0, 8, res[8 * j:8 * j + 8])

    def out_copy(g):
        segs = pl.ds(g * 4, 4)
        return pltpu.make_async_copy(obuf.at[segs], out_hbm.at[segs], osems.at[g])

    def group(g, mem, filler):
        plan = FILL_PLAN if filler else ((), (), (), ())
        for j in range(4):
            for n in plan[j]:
                oproj_b(g - 1, n)
            mem = step(4 * g + j, mem)
        if filler:
            finish_b(g - 1)
            out_copy(g - 1).start()
        return mem

    with jax.named_scope("group0"):
        mem = group(0, mem0_ref[...].astype(f32), False)
    with jax.named_scope("loop"):
        lax.fori_loop(1, NSEG // 4, lambda g, m: group(g, m, True), mem)
    with jax.named_scope("tail"):
        for n in range(KT):
            oproj_b(NSEG // 4 - 1, n)
        finish_b(NSEG // 4 - 1)
        out_copy(NSEG // 4 - 1).start()
    with jax.named_scope("wait_out"):
        for g in range(NSEG // 4):
            out_copy(g).wait()


@functools.partial(jax.jit, static_argnames=("A_seg_len",))
def pallas_recurrent_scan__memory_aug_recurrent_mem_tr__moe_arch_mod__prompt_kernel(
    A_x: jax.Array,
    A_mem0: jax.Array,
    A_Wq: jax.Array,
    A_Wk: jax.Array,
    A_Wv: jax.Array,
    A_Wo: jax.Array,
    A_seg_len,
    B_x: jax.Array,
    B_w_r: jax.Array,
    B_w_gate: jax.Array,
    B_w_up: jax.Array,
    B_w_down: jax.Array,
):
    del B_x
    assert A_seg_len == SEG
    assert A_x.shape == (1, S, D) and A_Wq.shape == (D, H, E) and B_w_gate.shape == (D, F)
    hbm = pl.BlockSpec(memory_space=pl.ANY)
    vmem = pl.BlockSpec(memory_space=pltpu.VMEM)
    out = pl.pallas_call(
        _kernel,
        out_shape=jax.ShapeDtypeStruct((NSEG, SEG, D), bf16),
        in_specs=[hbm, vmem, hbm, hbm, hbm, hbm, vmem, hbm, hbm, hbm],
        out_specs=hbm,
        scratch_shapes=[
            pltpu.VMEM((NSEG, SEG, D), bf16),
            pltpu.VMEM((NSEG, 24, D), f32),
            pltpu.VMEM((S, D), f32),
            pltpu.VMEM((NSEG * 4, D), u32),
            pltpu.VMEM((16, D), f32),
            pltpu.VMEM((16, F), f32),
            pltpu.VMEM((NCH, D, 8, E), bf16),
            pltpu.VMEM((KT, H * E, 128), bf16),
            pltpu.VMEM((3, NP, NSEG, 8, E), u32),
            pltpu.VMEM((H, NSEG * 8, E), f32),
            pltpu.VMEM((F, D), bf16),
            pltpu.VMEM((F, D), bf16),
            pltpu.VMEM((F, D), bf16),
            pltpu.VMEM((NSEG, SEG, D), bf16),
            pltpu.VMEM((KT, 32, 128), f32),
            pltpu.VMEM((KT, 32, 128), f32),
            pltpu.SemaphoreType.DMA((22,)),
            pltpu.SemaphoreType.DMA((NSEG // 4,)),
        ] + [pltpu.VMEM((2, 4 * PITCH, E), u32)] * NCH,
        compiler_params=pltpu.CompilerParams(vmem_limit_bytes=120 * 1024 * 1024),
    )(A_x.reshape(NSEG, SEG, D), A_mem0.reshape(M, D), A_Wq, A_Wk, A_Wv, A_Wo.reshape(H * E, D),
      B_w_r, B_w_gate.T, B_w_up.T, B_w_down)
    return out.reshape(1, S, D)
```

```python
import functools

import jax
import jax.numpy as jnp
from jax import lax
import jax.experimental.pallas as pl
import jax.experimental.pallas.tpu as pltpu

bf16 = jnp.bfloat16
f32 = jnp.float32
u32 = jnp.uint32

S, D, H, E = 2048, 640, 32, 128
M, SEG = 8, 32
NSEG = S // SEG
NP = H // 2
F, C = 1728, 8
KT = D // 128
NCH = 12
PITCH = 328
EPS_BF16 = 1.0013580322265625e-05
KEY0 = 0x3F800000
NT = (((1,), (1,)), ((), ()))

DQK, DPV, SPLIT = 1, 3, 13
DMX = int(0); DEX = int(0); DNM = int(0)
GEN = int(32); SIG = int(1)
OPQ = int(0)
SM = int('0'); DV = int('2')
CAT = int('2')
ORD = 'kqv'
GSL0 = [int(v) for v in '0,1,2,3,4'.split(',')]
GSL = [int(v) for v in '0,0,5,10,15'.split(',')]
POS = [int(v) for v in '15,30'.split(',')]
LNB, LNA = 8, int(8)
RL0 = int(4)
TRIM = int('1'); NOCHK = int(3); PRIO = ''
FFNF = int(1); FKC = int(4)
DEADL = int(0)
ONEP = int(0); LNORD = int(0)
LNFAST = int(1); LNSPLIT = int(192)
LNA_LAG = tuple(int(c) for c in '0011')
PRE = int(1)
MODE = 'std'
U = int(4)
FILL_PLAN = ((), (0, 1), (2, 3), (4,))


def _rb(v):
    return v.astype(bf16).astype(f32)


def _masks():
    r = lax.broadcasted_iota(jnp.int32, (80, 80), 0)
    c = lax.broadcasted_iota(jnp.int32, (80, 80), 1)

    def head(i):
        return jnp.where(i < 64, i >> 5, (i - 64) >> 3)

    def pos(i):
        j = i & 31
        return jnp.where(i < 64, jnp.where(j < 8, j, j + 8), 8 + (i & 7))

    same = head(r) == head(c)
    pr, pc = pos(r), pos(c)
    keep = same & ((pr < M) | (pr >= pc))
    fill = jnp.where(same, -1000000000.0, -jnp.inf).astype(f32)
    return keep, fill


def _interleave(units, side):
    done = 0
    for i, unit in enumerate(units):
        unit()
        want = (len(side) * (i + 1)) // len(units)
        for task in side[done:want]:
            task()
        done = want


def _kernel(x_hbm, mem0_hbm, wq_hbm, wk_hbm, wv_hbm, wo_hbm, wr_hbm, wg_hbm, wu_hbm, wd_hbm,
            out_hbm,
            xbuf, xa32, xb32, xnb, sel_ref, hh_ref, wraw, wo, qkvb, ob,
            wg, wu, wd, obuf, accs, accb, oa, obr, mem0_ref, wr_ref, sems, osems, *rest):
    wqkv, accg = rest[:NCH], rest[NCH:]
    w_hbm = (wq_hbm, wk_hbm, wv_hbm)

    cp_xb = pltpu.make_async_copy(x_hbm.at[:, pl.ds(0, 8), :], xbuf.at[:, pl.ds(0, 8), :],
                                  sems.at[0])
    cp_xa = pltpu.make_async_copy(x_hbm.at[:, pl.ds(8, 24), :], xbuf.at[:, pl.ds(8, 24), :],
                                  sems.at[1])
    cp_w = [pltpu.make_async_copy(w_hbm[c // 4].at[:, pl.ds(8 * (c % 4), 8), :], wraw.at[c],
                                  sems.at[2 + c]) if c else None for c in range(NCH)]
    cp_ffn = [pltpu.make_async_copy(src, dst, sems.at[14 + i])
              for i, (src, dst) in enumerate(((wg_hbm, wg), (wu_hbm, wu), (wd_hbm, wd)))]
    cp_wo = [pltpu.make_async_copy(wo_hbm.at[:, pl.ds(128 * n, 128)], wo.at[n], sems.at[17 + n])
             for n in range(KT)]
    cp_w0 = [pltpu.make_async_copy(wq_hbm.at[pl.ds(128 * k, 128), pl.ds(0, 8), :],
                                   wraw.at[0, pl.ds(128 * k, 128)], sems.at[22 + k])
             for k in range(KT)]
    cp_wr = pltpu.make_async_copy(wr_hbm, wr_ref, sems.at[27])
    cp_m0 = pltpu.make_async_copy(mem0_hbm, mem0_ref.at[pl.ds(0, 8)], sems.at[28])
    for i, cp in enumerate([cp_xb, cp_wr] + cp_w0 + cp_w[1:7] + [cp_xa] + cp_w[7:] + cp_ffn + cp_wo
                           + [cp_m0]):
        cp.start(priority=int(PRIO[i]) if i < len(PRIO) else int(PRIO[-1:] or 0))
    cp_xb.wait()
    cp_wr.wait()

    wr = wr_ref[...].astype(f32).reshape(1, D)
    wsum = jnp.sum(wr, axis=-1, keepdims=True)
    lane = lax.broadcasted_iota(jnp.int32, (8, 128), 1)
    scores = [jnp.zeros((8, 128), f32), jnp.zeros((8, 128), f32)]

    tokens = []

    def layernorm(batches, lag):
        st = {}
        n = len(batches)

        def load(i):
            return jnp.concatenate(
                [xbuf[g // 4, 8 * (g % 4):8 * (g % 4) + 8, :].astype(f32) for g in batches[i]], axis=0)

        def mean(i):
            x = load(i)
            st['mu', i] = jnp.mean(x, axis=-1, keepdims=True)
            if ONEP:
                st['xx', i] = jnp.mean(x * x, axis=-1, keepdims=True)
                st['xw', i] = jnp.sum(x * wr, axis=-1, keepdims=True)

        def var(i):
            if ONEP:
                st['var', i] = jnp.maximum(st['xx', i] - st['mu', i] * st['mu', i], 0.0)
                return
            xc = load(i) - st['mu', i]
            st['var', i] = jnp.mean(xc * xc, axis=-1, keepdims=True)

        def norm(i):
            v = _rb(_rb(st['var', i]) + EPS_BF16)
            if LNFAST:
                den = _rb(v * lax.rsqrt(v))
                inv = pl.reciprocal(den, approx=True)
                inv = inv * (2.0 - den * inv)
                xn = (load(i) - _rb(st['mu', i])) * inv
            else:
                den = _rb(jnp.sqrt(v))
                xn = _rb(_rb(load(i) - _rb(st['mu', i])) * (1.0 / den))
            for k, g in enumerate(batches[i]):
                xb32[8 * g:8 * g + 8, :] = xn[8 * k:8 * k + 8]
                if g % 4:
                    xa32[g // 4, 8 * (g % 4) - 8:8 * (g % 4), :] = xn[8 * k:8 * k + 8]
            if batches[i][0] % 4 == 0:
                s0 = batches[i][0] // 4
                xnb[4 * s0:4 * (s0 + len(batches[i])), :] = pltpu.bitcast(xn.astype(bf16), u32)
            if ONEP:
                st['r', i] = (st['xw', i] - _rb(st['mu', i]) * wsum) * inv
            else:
                st['r', i] = jnp.sum(xn * wr, axis=-1, keepdims=True)

        def score(i):
            if DEADL and batches[i][0] % 4:
                tot = st['r', i][0:8]
                for k in range(1, len(batches[i])):
                    tot = tot + st['r', i][8 * k:8 * k + 8]
                tokens.append(tot)
            for k, g in enumerate(batches[i]):
                scores[g // 128] = jnp.where(lane == g % 128, st['r', i][8 * k:8 * k + 8],
                                             scores[g // 128])

        def stage(t):
            for d, fn in zip(lag, (mean, var, norm, score)):
                if 0 <= t - d < n:
                    fn(t - d)

        return [functools.partial(stage, t) for t in range(n + lag[-1])]

    def chunks(v, k):
        return [v[i:i + k] for i in range(0, len(v), k)]

    ln_b = layernorm(chunks([4 * sg for sg in range(NSEG)], LNB), (0, 1, 2, 3))
    a_groups = [g for g in range(4 * NSEG) if g % 4]
    ln_a1 = layernorm(chunks(a_groups[:LNSPLIT], LNA), LNA_LAG)
    ln_a2 = layernorm(chunks(a_groups[LNSPLIT:], LNA), LNA_LAG) if LNSPLIT < 192 else []

    def relayout(c, i):
        for dd in range(16 * i, 16 * i + 16):
            a = pltpu.bitcast(wraw[c, 2 * dd], u32)
            b = pltpu.bitcast(wraw[c, 2 * dd + 1], u32)
            rows = pl.ds(dd, 4, stride=PITCH)
            wqkv[c][0, rows, :] = (a & jnp.uint32(0xFFFF)) | (b << 16)
            wqkv[c][1, rows, :] = (a >> 16) | (b & jnp.uint32(0xFFFF0000))

    def wtile(t, par, hp):
        start = (hp % 4) * PITCH
        w = wqkv[4 * t + hp // 4][par, start:start + D // 2, :]
        return pltpu.bitcast(w, bf16)

    def prepass(c, p, mb):
        t, hp = c // 4, (c % 4) * 4 + p
        lhs = xnb[mb * 64:(mb + 1) * 64, :]
        if len(tokens) >= DEADL > 0:
            z = pltpu.bitcast(jnp.broadcast_to(tokens.pop(0), (8, 128)), u32)
            z = (z >> 16) >> 16
            top = jnp.concatenate([lhs[0:8, 0:128] | z, lhs[0:8, 128:]], axis=1)
            lhs = jnp.concatenate([top, lhs[8:]], axis=0)
        lhs = pltpu.bitcast(lhs, bf16)
        y0 = jnp.dot(lhs, wtile(t, 0, hp), preferred_element_type=f32).reshape(16, 8, E)
        y1 = jnp.dot(lhs, wtile(t, 1, hp), preferred_element_type=f32).reshape(16, 8, E)
        y = jnp.concatenate([y0, y1], axis=1).astype(bf16)
        qkvb[t, hp, mb * 16:(mb + 1) * 16] = pltpu.bitcast(y, u32)

    route = {}

    def top_c():
        r = _rb(jnp.concatenate(scores, axis=1)) + 0.0
        tok = (lax.broadcasted_iota(jnp.int32, (8, 256), 1) * 8
               + lax.broadcasted_iota(jnp.int32, (8, 256), 0))
        bits = lax.shift_right_logical(pltpu.bitcast(r, jnp.int32), 16)
        rank = jnp.where(bits >= 0x8000, 0xFFFF - bits, bits + 0x8000)
        rank = jnp.where(r == r, rank, 0)
        key = pltpu.bitcast(rank * 2048 + (S - 1 - tok) + KEY0, f32)
        row16 = lax.broadcasted_iota(jnp.int32, (16, 128), 0)
        sel_ref[8:16, :] = jnp.zeros((8, D), f32)
        picked = jnp.full((16, 128), KEY0 + 0x8000 * 2048, jnp.int32)
        idxs = []
        for j in range(C):
            best = jnp.max(key, keepdims=True)
            key = jnp.where(key == best, 0.0, key)
            code = pltpu.bitcast(jnp.broadcast_to(best, (16, 128)), jnp.int32)
            picked = jnp.where(row16 == j, code, picked)
            idx = (S - 1) - ((code[0, 0] - KEY0) & (S - 1))
            idxs.append(idx)
            sel_ref[j:j + 1, :] = xb32[pl.ds(idx, 1), :]
        rank = lax.shift_right_logical(picked - KEY0, 11)
        bits = jnp.where(rank >= 0x8000, rank - 0x8000, 0xFFFF - rank)
        route['idx'] = idxs
        route['gate'] = jax.nn.sigmoid(pltpu.bitcast(bits << 16, f32))

    def ffn_up(n):
        cols = slice(128 * n, min(128 * (n + 1), F))
        xsb = sel_ref[0:16, :].astype(bf16)
        hg = lax.dot_general(xsb, wg[cols, :], NT, preferred_element_type=f32)
        hu = lax.dot_general(xsb, wu[cols, :], NT, preferred_element_type=f32)
        hh_ref[:, cols] = hg * jax.nn.sigmoid(hg) * hu

    def ffn_down(n):
        cols = slice(128 * n, 128 * (n + 1))
        y = jnp.dot(hh_ref[...].astype(bf16), wd[:, cols], preferred_element_type=f32)
        sel_ref[0:16, cols] = sel_ref[0:16, cols] + y * route['gate']

    def ffn_gate(n):
        cols = slice(128 * n, min(128 * (n + 1), F))
        hg = lax.dot_general(sel_ref[0:16, :].astype(bf16), wg[cols, :], NT,
                             preferred_element_type=f32)
        route['g', n] = hg * jax.nn.sigmoid(hg)

    def ffn_up2(n):
        cols = slice(128 * n, min(128 * (n + 1), F))
        hu = lax.dot_general(sel_ref[0:16, :].astype(bf16), wu[cols, :], NT,
                             preferred_element_type=f32)
        hh_ref[:, cols] = route['g', n] * hu

    def ffn_down2(n, k0):
        cols = slice(128 * n, 128 * (n + 1))
        ks = slice(128 * k0, min(128 * (k0 + FKC), F))
        y = jnp.dot(hh_ref[:, ks].astype(bf16), wd[ks, cols], preferred_element_type=f32)
        sel_ref[16:32, cols] = sel_ref[(16 if k0 else 0):(32 if k0 else 16), cols] + y * route['gate']

    def ffn_scatter():
        for j in range(C):
            xb32[pl.ds(route['idx'][j], 1), :] = sel_ref[(16 if FFNF else 0) + j:(16 if FFNF else 0) + j + 1, :]

    P = functools.partial
    pp = lambda c, ps=range(4): [P(prepass, c, p, mb) for p in ps for mb in range(4)]
    rl = lambda c: [P(relayout, c, i) for i in range(20)]

    def block(name, waits, units, side):
        with jax.named_scope("wait_" + name):
            for cp in waits:
                cp.wait()
        with jax.named_scope("blk_" + name):
            if PRE:
                _interleave(units, side)

    block("lnb", [], ln_b, [])
    block("rl0", cp_w0[:RL0], rl(0)[:4 * RL0], [])
    block("0", cp_w0[RL0:], rl(0)[4 * RL0:] + pp(0, (0, 1)), [])
    block("1", cp_w[1:2], pp(0, (2, 3)), rl(1))
    block("2", cp_w[2:3], pp(1), rl(2))
    block("3", cp_w[3:5], pp(2), rl(3) + rl(4))
    block("4", cp_w[5:7], pp(3) + pp(4), rl(5) + rl(6))
    block("5", [cp_xa] + cp_w[7:9], pp(5) + pp(6), (ln_a1 + rl(7) + rl(8)) if LNORD == 0 else (rl(7) + rl(8) + ln_a1) if LNORD == 1 else ([lambda: [t() for t in rl(7) + rl(8)]] + ln_a1))
    tokens.clear()
    block("6", cp_w[9:12], pp(7) + pp(8), ln_a2 + [top_c] + rl(9) + rl(10) + rl(11))
    block("7", cp_ffn, pp(9) + pp(10) + pp(11),
          [P(ffn_up, n) for n in range(14)] + [P(ffn_down, n) for n in range(KT)] + [ffn_scatter]
          if not FFNF else
          [P(f, n) for n in range(14) for f in (ffn_gate, ffn_up2)]
          + [P(ffn_down2, n, k0) for k0 in range(0, 14, FKC) for n in range(KT)]
          + [ffn_scatter] + [lambda: None] * (FFNF - 1))
    block("wo", cp_wo + [cp_m0], [], [])

    def finish(s, lo, n, s_val):
        r0 = s * SEG if isinstance(s, int) else pl.multiple_of(s * SEG, SEG)
        b = xb32[pl.ds(r0 + lo, n), :]
        x = xbuf[s, lo:lo + n, :].astype(f32)
        hb = 0.5 * b
        g = (hb * jnp.tanh(hb) + hb) if SIG else b * jax.nn.sigmoid(b)
        obuf[s, lo:lo + n, :] = (x + s_val * g).astype(bf16)

    keep, fill = _masks()
    c80 = lax.broadcasted_iota(jnp.int32, (8, 80), 1)
    r80 = lax.broadcasted_iota(jnp.int32, (8, 80), 0)
    is_h0 = (c80 < 32) | ((c80 >= 64) & (c80 < 72))
    is_h1 = jnp.logical_not(is_h0)
    cj = c80 & 31
    cpos = jnp.where(c80 < 64, jnp.where(cj < 8, cj, cj + 8), 8 + (c80 & 7))
    causal = [None] + [cpos <= r80 + 8 + 8 * i for i in (1, 2, 3)] + [cpos <= r80 + 8]
    grp = [(0, 4), (1, 5), (2, 6), (3, 7), (8, 9)]
    scale = E ** -0.5

    def step(s, j, mem, gen=None, pre_finish=None):
        lhs = jnp.concatenate([mem, xa32[s]], axis=0).astype(bf16)
        st = {}
        z1 = s >> 10
        z2 = [s >> (11 + n) for n in range(KT)]

        def proj(hp, t, par, k0, k1):
            start = (hp % 4) * PITCH
            w = pltpu.bitcast(wqkv[4 * t + hp // 4][par, start + 64 * k0:start + 64 * k1, :], bf16)
            y = jnp.dot(lhs[:, 128 * k0:128 * k1], w, preferred_element_type=f32)
            if k0 > 0:
                y = jnp.maximum(st["y", hp, t, par], -3.0e38) + y
            st['y', hp, t, par] = y
            if par == 1 and k1 == KT:
                y0, y1 = st['y', hp, t, 0], y
                if CAT == 0:
                    yb = pltpu.bitcast(qkvb[t, hp, s], bf16)
                    r = jnp.concatenate([y0.astype(bf16), y1.astype(bf16), yb], axis=0)
                elif CAT >= 2:
                    yb = pltpu.bitcast(qkvb[t, hp, s], bf16).astype(f32)
                    r = jnp.concatenate([y0, y1, yb], axis=0).astype(bf16)
                else:
                    ya = pltpu.bitcast(jnp.concatenate([y0, y1], axis=0).astype(bf16), u32)
                    r = pltpu.bitcast(jnp.concatenate([ya, qkvb[t, hp, s]], axis=0), bf16)
                st['qkv', hp, t] = r

        def qk(hp):
            q, k = st['qkv', hp, 0], st['qkv', hp, 1]
            sc = lax.dot_general(q, k, NT, preferred_element_type=f32)
            if SM == 0:
                sc = jnp.where(keep, sc * scale, fill)
                p = jnp.exp(sc - jnp.max(sc, axis=-1, keepdims=True))
                l = jnp.sum(p, axis=-1, keepdims=True)
                st['p', hp] = (p * pl.reciprocal(l, approx=True)).astype(bf16)
                return
            rows = [None] * 10
            for i, (g0, g1) in enumerate(grp):
                s0, s1 = sc[8 * g0:8 * g0 + 8], sc[8 * g1:8 * g1 + 8]
                if SM == 1:
                    for g, sg, hm in ((g0, s0, is_h0), (g1, s1, is_h1)):
                        sg = sg * scale
                        if causal[i] is not None:
                            sg = jnp.where(causal[i], sg, -1000000000.0)
                        sg = jnp.where(hm, sg, -jnp.inf)
                        e = jnp.exp(sg - jnp.max(sg, axis=-1, keepdims=True))
                        l = jnp.sum(e, axis=-1, keepdims=True)
                        rows[g] = e * pl.reciprocal(l, approx=True)
                else:
                    sm = jnp.where(is_h0, s0, s1) * scale
                    if causal[i] is not None:
                        sm = jnp.where(causal[i], sm, -1000000000.0)
                    m0 = jnp.max(jnp.where(is_h0, sm, -jnp.inf), axis=-1, keepdims=True)
                    m1 = jnp.max(jnp.where(is_h0, -jnp.inf, sm), axis=-1, keepdims=True)
                    e = jnp.exp(sm - jnp.where(is_h0, m0, m1))
                    l0 = jnp.sum(jnp.where(is_h0, e, 0.0), axis=-1, keepdims=True)
                    l1 = jnp.sum(jnp.where(is_h0, 0.0, e), axis=-1, keepdims=True)
                    if SM == 2:
                        pn = e * pl.reciprocal(jnp.where(is_h0, l0, l1), approx=True)
                        rows[g0] = jnp.where(is_h0, pn, 0.0)
                        rows[g1] = jnp.where(is_h0, 0.0, pn)
                    else:
                        rows[g0] = e * jnp.where(is_h0, pl.reciprocal(l0, approx=True), 0.0)
                        rows[g1] = e * jnp.where(is_h0, 0.0, pl.reciprocal(l1, approx=True))
            st['p', hp] = jnp.concatenate(rows, axis=0).astype(bf16)

        def pv(hp):
            o = jnp.dot(st['p', hp], st['qkv', hp, 2], preferred_element_type=f32)
            if OPQ & 1 and hp < SPLIT:
                oa[z1 + hp] = pltpu.bitcast(o[0:64].astype(bf16), u32)
            elif CAT >= 3:
                st['o', 2 * hp] = o[0:32]
                st['o', 2 * hp + 1] = o[32:64]
            else:
                st['o', 2 * hp] = o[0:32].astype(bf16)
                st['o', 2 * hp + 1] = o[32:64].astype(bf16)
            rb = pl.ds(8 * j, 8)
            ob[2 * hp, rb, :] = o[64:72]
            ob[2 * hp + 1, rb, :] = o[72:80]

        def oproj(n, h0, h1):
            if OPQ & 1 and h0 == 0:
                zz = z2[n] if OPQ & 4 else z2[0]
                a = jnp.concatenate([pltpu.bitcast(oa[zz + h // 2, 16 * (h % 2):16 * (h % 2) + 16], bf16)
                                     for h in range(h0, h1)], axis=1)
            else:
                a = jnp.concatenate([st['o', h] for h in range(h0, h1)], axis=1).astype(bf16)
            w = wo[n, h0 * 128:h1 * 128, :]
            return jnp.dot(a, w, preferred_element_type=f32)

        def at(fn, t, d):
            if 0 <= t - d < NP:
                fn(t - d)

        nop = 0
        for t in range(NP + KT + DV):
            if gen is not None:
                for u in gen.get(t, ()):
                    u()
            cuts = sorted(set(range(0, 31, 5)) | set(POS))
            for i, c in enumerate(cuts):
                if POS[0] == c:
                    at(qk, t, DQK)
                if POS[1] == c:
                    at(pv, t, DPV)
                if c < 30:
                    u = c // 5
                    which = 'qkv'.index(ORD[u // 2])
                    tt = t - DV if which == 2 else t
                    if 0 <= tt < NP:
                        proj(tt, which, u % 2, c - 5 * u, cuts[i + 1] - 5 * u)
                    if t >= NP and c == 0 and nop < KT:
                        accs[nop] = oproj(nop, 0, 2 * SPLIT)
                        nop += 1
        acc = jnp.concatenate([accs[n] + oproj(n, 2 * SPLIT, H) for n in range(KT)], axis=1)
        if pre_finish is not None:
            pre_finish()
        finish(s, 8, 24, acc[8:32])
        return _rb(acc[0:8])

    def dyn(v, m):
        return v if isinstance(v, int) else pl.multiple_of(v, m)

    def oproj_b(slot, nslots, h0, nh, n):
        rows = pl.ds(dyn(slot * 16, 16), 16 * nslots)
        a = jnp.concatenate([pltpu.bitcast(obr[h0 + i, rows, :], bf16) for i in range(nh)], axis=1)
        w = wo[n, pl.ds(dyn(h0 * 128, 128), nh * 128), :]
        return jnp.dot(a, w, preferred_element_type=f32)

    def finish_b(g, res):
        for j in range(4):
            finish(g * 4 + j, 0, 8, res[8 * j:8 * j + 8])

    def out_copy(g):
        segs = pl.ds(g * 4, 4)
        return pltpu.make_async_copy(obuf.at[segs], out_hbm.at[segs], osems.at[g])

    def pack_b(g):
        for h in range(H):
            obr[h, pl.ds(dyn((g + 1) * 16, 16), 16), :] = pltpu.bitcast(ob[h].astype(bf16), u32)

    def group(g, mem, filler):
        if filler:
            pack_b(g - 1)
        for j in range(4):
            gen = {}
            if filler:
                def unit(n, j=j):
                    r = oproj_b(g - 1, 2, (g % 2) * 16 + 4 * j, 4, n)
                    if OPQ & 2:
                        accg[n][g >> (10 + j)] = r if j == 0 else accg[n][g >> (20 + j)] + r
                    else:
                        accg[n][0] = r if j == 0 else accg[n][0] + r
                for n, sl in enumerate(GSL0 if j == 0 else GSL):
                    gen.setdefault(sl, []).append(P(unit, n))
            mem = step(4 * g + j, j, mem, gen)
        if filler:
            zg = g >> 28 if OPQ & 2 else 0
            done = jnp.concatenate([accb[n] + accg[n][zg, 0:32] for n in range(KT)], axis=1)
            finish_b(jnp.maximum(g - 2, 0), done)
            for n in range(KT):
                accb[n] = accg[n][zg, 32:64]

            @pl.when(g >= 2)
            def _():
                out_copy(g - 2).start()
        return mem

    def group32(g, mem, filler):
        if filler and TRIM & 2:
            @pl.when(g >= 2)
            def _():
                out_copy(g - 2).start()
        prev = [ob[h] if CAT >= 4 else ob[h].astype(bf16) for h in range(H)] if filler else None

        def fin_b():
            finish_b(g - 1, jnp.concatenate([accb[n] for n in range(KT)], axis=1))

        for j in range(4):
            gen = {}
            if filler:
                def unit(n, j=j):
                    a = jnp.concatenate(prev[8 * j:8 * j + 8], axis=1).astype(bf16)
                    r = jnp.dot(a, wo[n, 1024 * j:1024 * (j + 1), :], preferred_element_type=f32)
                    accb[n] = r if j == 0 else accb[n] + r
                for n, sl in enumerate(GSL0 if j == 0 else GSL):
                    gen.setdefault(sl, []).append(P(unit, n))
            mem = step(4 * g + j, j, mem, gen, fin_b if filler and j == 3 and TRIM & 1 else None)
        if filler:
            if not TRIM & 1:
                fin_b()
            if not TRIM & 2:
                out_copy(g - 1).start()
        return mem

    if GEN == 32:
        group = group32

    NG = NSEG // 4
    obr[:, 0:16, :] = jnp.zeros((H, 16, E), u32)
    accb[...] = jnp.zeros(accb.shape, f32)
    mem = mem0_ref[0:8, :].astype(f32)
    if MODE == 'u8':
        ob[...] = jnp.zeros(ob.shape, f32)

        def body8(i, m):
            m = group(2 * i, m, 2)
            m = group(2 * i + 1, m, 3)

            @pl.when(i >= 1)
            def _():
                out_copy(2 * i - 1).start()
            out_copy(2 * i).start()
            return m
        with jax.named_scope("loop"):
            lax.fori_loop(0, NG // 2, body8, mem)
    if MODE == 'std':
        with jax.named_scope("group0"):
            mem = group(0, mem, False)
    if MODE == 'u8':
        pass
    elif MODE != 'noloop':
        with jax.named_scope("loop"):
            def body(g, m):
                return group(g, m, True)
            if None:
                lax.fori_loop(1, NG // 2, lambda i, m: body(2 * i + 1, body(2 * i, m)), mem)
            else:
                lax.fori_loop(1, NG, body, mem)
    else:
        for g in range(NG - (2 if GEN == 64 else 1)):
            out_copy(g).start()
    with jax.named_scope("tail"):
        if GEN == 64:
            pack_b(NG - 1)
            lo = [oproj_b(NG - 1, 2, 0, 16, n) for n in range(KT)]
            finish_b(NG - 2, jnp.concatenate([accb[n] + lo[n][0:32] for n in range(KT)], axis=1))
            out_copy(NG - 2).start()
            hi = [oproj_b(NG, 1, 16, 16, n) for n in range(KT)]
            finish_b(NG - 1, jnp.concatenate([hi[n] + lo[n][32:64] for n in range(KT)], axis=1))
            out_copy(NG - 1).start()
        else:
            if TRIM & 2:
                out_copy(NG - 2).start()
            a = jnp.concatenate([ob[h].astype(bf16) for h in range(H)], axis=1)
            finish_b(NG - 1, jnp.concatenate(
                [jnp.dot(a, wo[n], preferred_element_type=f32) for n in range(KT)], axis=1))
            out_copy(NG - 1).start()
    with jax.named_scope("wait_out"):
        for g in range(NG):
            out_copy(g).wait()


@functools.partial(jax.jit, static_argnames=("A_seg_len",))
def pallas_recurrent_scan__memory_aug_recurrent_mem_tr__moe_arch_mod__prompt_kernel(
    A_x: jax.Array,
    A_mem0: jax.Array,
    A_Wq: jax.Array,
    A_Wk: jax.Array,
    A_Wv: jax.Array,
    A_Wo: jax.Array,
    A_seg_len,
    B_x: jax.Array,
    B_w_r: jax.Array,
    B_w_gate: jax.Array,
    B_w_up: jax.Array,
    B_w_down: jax.Array,
):
    del B_x
    assert A_seg_len == SEG
    assert A_x.shape == (1, S, D) and A_Wq.shape == (D, H, E) and B_w_gate.shape == (D, F)
    hbm = pl.BlockSpec(memory_space=pl.ANY)
    vmem = pl.BlockSpec(memory_space=pltpu.VMEM)
    out = pl.pallas_call(
        _kernel,
        out_shape=jax.ShapeDtypeStruct((NSEG, SEG, D), bf16),
        in_specs=[hbm] * 10,
        out_specs=hbm,
        scratch_shapes=[
            pltpu.VMEM((NSEG, SEG, D), bf16),
            pltpu.VMEM((NSEG, 24, D), f32),
            pltpu.VMEM((S, D), f32),
            pltpu.VMEM((NSEG * 4, D), u32),
            pltpu.VMEM((32, D), f32),
            pltpu.VMEM((16, F), f32),
            pltpu.VMEM((NCH, D, 8, E), bf16),
            pltpu.VMEM((KT, H * E, 128), bf16),
            pltpu.VMEM((3, NP, NSEG, 8, E), u32),
            pltpu.VMEM((H, 32, E), f32),
            pltpu.VMEM((F, D), bf16),
            pltpu.VMEM((F, D), bf16),
            pltpu.VMEM((F, D), bf16),
            pltpu.VMEM((NSEG, SEG, D), bf16),
            pltpu.VMEM((KT, 32, 128), f32),
            pltpu.VMEM((KT, 32, 128), f32),
            pltpu.VMEM((NP, 32, 128), u32),
            pltpu.VMEM((H, (NSEG // 4 + 1) * 16, E), u32),
            pltpu.VMEM((64, D), bf16),
            pltpu.VMEM((D,), bf16),
            pltpu.SemaphoreType.DMA((29,)),
            pltpu.SemaphoreType.DMA((NSEG // 4,)),
        ] + [pltpu.VMEM((2, 4 * PITCH, E), u32)] * NCH + [pltpu.VMEM((1, 64, 128), f32)] * KT,
        compiler_params=pltpu.CompilerParams(vmem_limit_bytes=120 * 1024 * 1024,
            disable_bounds_checks=bool(NOCHK & 1), disable_semaphore_checks=bool(NOCHK & 2)),
    )(A_x.reshape(NSEG, SEG, D), A_mem0.reshape(M, D), A_Wq, A_Wk, A_Wv, A_Wo.reshape(H * E, D),
      B_w_r, B_w_gate.T, B_w_up.T, B_w_down)
    return out.reshape(1, S, D)
```

```python
import functools

import jax
import jax.numpy as jnp
from jax import lax
import jax.experimental.pallas as pl
import jax.experimental.pallas.tpu as pltpu

bf16 = jnp.bfloat16
f32 = jnp.float32
u32 = jnp.uint32

S, D, H, E = 2048, 640, 32, 128
M, SEG = 8, 32
NSEG = S // SEG
NG = NSEG // 4
NP = H // 2
F, C = 1728, 8
KT = D // 128
NCH = 12
PITCH = 328
EPS_BF16 = 1.0013580322265625e-05
KEY0 = 0x3F800000
NT = (((1,), (1,)), ((), ()))

DQK, DPV, SPLIT = 1, 3, 13
SM = int(0)
DV = int(2)
CAT = int(2)
ORD = 'kqv'
POS = [int(v) for v in '3,6'.split(',')]
FILL = [(int(v.split(':')[0]), int(v.split(':')[1]))
        for v in '1:0,1:0,2:0,2:0,3:0,3:0'.split(',')]
NF = len(FILL)
LNB, LNA = 8, int(2)
LNA_LAG = tuple(int(c) for c in '0123')
PPM = int(128)
PPM7 = int(128)
FKC = int(5)
WGR = [[int(c) for c in g.split('.')] for g in '0.1.2.3.4.5.6.7.8.9.10.11'.split(',')]
EARLY = int(2); PPML = int(128)
CHK = int(1); OPW = int(1)
ONCE = '16'
XW = int(1024); GB = int(1); PLAN = int(3); TA = int(3); VFE = int(0); E7 = int(0); H0 = int(5); H1 = int(13)
ALIAS = int(1)
PRE = int(1)
MODE = 'std'


def _rb(v):
    return v.astype(bf16).astype(f32)


def _masks():
    r = lax.broadcasted_iota(jnp.int32, (80, 80), 0)
    c = lax.broadcasted_iota(jnp.int32, (80, 80), 1)

    def head(i):
        return jnp.where(i < 64, i >> 5, (i - 64) >> 3)

    def pos(i):
        j = i & 31
        return jnp.where(i < 64, jnp.where(j < 8, j, j + 8), 8 + (i & 7))

    same = head(r) == head(c)
    pr, pc = pos(r), pos(c)
    keep = same & ((pr < M) | (pr >= pc))
    fill = jnp.where(same, -1000000000.0, -jnp.inf).astype(f32)
    return keep, fill


def _aligned(v, m):
    return v if isinstance(v, int) else pl.multiple_of(v, m)


def _merge(a, b):
    keyed = [((i + 0.5) / len(a), 0, t) for i, t in enumerate(a)]
    keyed += [((i + 0.5) / len(b), 1, t) for i, t in enumerate(b)]
    return [t for _, _, t in sorted(keyed, key=lambda e: e[:2])]


def _interleave(units, side, early=0):
    done = 0
    for i, unit in enumerate(units):
        unit()
        want = min(len(side), (len(side) * (i + 1)) // (len(units) - early))
        for task in side[done:want]:
            task()
        done = want


def _kernel(x_hbm, mem0_hbm, wq_hbm, wk_hbm, wv_hbm, wo_hbm, wr_hbm, wg_hbm, wu_hbm, wd_hbm,
            out_hbm,
            xbuf, xa32, xb32, xnb, sel_ref, hh_ref, wraw, wo, qkvb, vnext,
            wg, wu, wd, obuf, accs, mem0_ref, sems, osems, *rest):
    wqkv, wr_ref = rest[:-1], rest[-1]
    P = functools.partial
    XA0 = 0
    if ALIAS:
        xa32, XA0 = qkvb, 3 * H
    w_hbm = (wq_hbm, wk_hbm, wv_hbm)

    def x_copy(j):
        return pltpu.make_async_copy(x_hbm.at[:, j], xbuf.at[:, j, :, pl.ds(0, D)], sems.at[25 + j])

    def w_copy(c, src):
        return pltpu.make_async_copy(src, wraw.at[c], sems.at[1 + c])

    cp_x = [x_copy(j) for j in range(4)]
    cp_w = [None] + [w_copy(c, w_hbm[c // 4].at[:, pl.ds(8 * (c % 4), 8), :])
                     for c in range(1, NCH)]
    cp_w0 = [pltpu.make_async_copy(wq_hbm.at[pl.ds(lo, n), pl.ds(0, 8), :],
                                   wraw.at[0, pl.ds(lo, n)], sems.at[13 + i])
             for i, (lo, n) in enumerate(((0, 512), (512, 128)))]
    cp_ffn = [pltpu.make_async_copy(src, dst, sems.at[15 + i])
              for i, (src, dst) in enumerate(((wg_hbm, wg), (wu_hbm, wu), (wd_hbm, wd)))]
    cp_wo = [pltpu.make_async_copy(wo_hbm.at[:, pl.ds(128 * n, 128)], wo.at[n], sems.at[18 + n])
             for n in range(KT)]
    cp_wr = pltpu.make_async_copy(wr_hbm, wr_ref, sems.at[23])
    cp_m0 = pltpu.make_async_copy(mem0_hbm, mem0_ref.at[pl.ds(0, 8)], sems.at[24])
    o1, o2, o3 = (3, 5, 7) if PLAN == 1 else (6, 8, 10)
    order = ([cp_x[0], cp_wr] + cp_w0 + cp_w[1:o1] + [cp_x[1]] + cp_w[o1:o2] + [cp_x[2]]
             + cp_w[o2:o3] + [cp_x[3]] + cp_w[o3:] + cp_ffn + cp_wo + [cp_m0])
    if PLAN == 3:
        order = ([cp_x[0], cp_wr] + cp_w0 + cp_w[1:6] + [cp_x[1]] + cp_w[6:8] + [cp_x[2], cp_w[10]]
                 + cp_w[8:10] + [cp_x[3], cp_w[11]] + cp_ffn + cp_wo + [cp_m0])
    for cp in order:
        cp.start()
    zero = lax.fori_loop(0, 2, lambda i, c: (c + i) >> 1, 0)
    cp_x[0].wait()
    cp_wr.wait()

    wr = wr_ref[...].astype(f32).reshape(1, D)
    lane = lax.broadcasted_iota(jnp.int32, (8, 128), 1)
    scores = [jnp.zeros((8, 128), f32), jnp.zeros((8, 128), f32)]

    def layernorm(j, s0, n, nb, lag, first):
        st = {}
        lane_j = lane - j

        def load(i):
            return xbuf[pl.ds(s0 + nb * i, nb), j, :, 0:D].astype(f32).reshape(8 * nb, D)

        def mean(i):
            st['mu', i] = jnp.mean(load(i), axis=-1, keepdims=True)

        def var(i):
            xc = load(i) - st['mu', i]
            st['var', i] = jnp.mean(xc * xc, axis=-1, keepdims=True)

        def norm(i):
            v = _rb(_rb(st['var', i]) + EPS_BF16)
            den = _rb(v * lax.rsqrt(v))
            inv = pl.reciprocal(den, approx=True)
            inv = inv * (2.0 - den * inv)
            xn = (load(i) - _rb(st['mu', i])) * inv
            xb32[pl.ds(s0 + nb * i, nb), j] = xn.reshape(nb, 8, D)
            if first:
                xnb[4 * nb * i:4 * nb * (i + 1), :] = pltpu.bitcast(xn.astype(bf16), u32)
            else:
                rows = pl.ds(_aligned(8 * (s0 + nb * i), 8), 8 * nb)
                for k in range(KT):
                    xa32[XA0 + KT * j + k, rows, :] = xn[:, 128 * k:128 * (k + 1)]
            st['r', i] = jnp.sum(xn * wr, axis=-1, keepdims=True)

        def score(i):
            for k in range(nb):
                sg = s0 + nb * i + k
                scores[sg // 32] = jnp.where(lane_j == 4 * (sg % 32), st['r', i][8 * k:8 * k + 8],
                                             scores[sg // 32])
            if CHK and not first:
                qkvb[3 * H + 4 * KT, 0:8, :] = scores[s0 // 32]

        def stage(t):
            for d, fn in zip(lag, (mean, var, norm, score)):
                if 0 <= t - d < n:
                    fn(t - d)

        return [P(stage, t) for t in range(n + lag[-1])]

    where = {c: (wqkv[k], i) for k, g in enumerate(WGR) for i, c in enumerate(g)}

    def relayout(c, i, it=0):
        ref, k = where[c]
        for dd in range(16 * i, 16 * i + 16):
            a = pltpu.bitcast(wraw[c + it, 2 * dd], u32)
            b = pltpu.bitcast(wraw[c + it, 2 * dd + 1], u32)
            rows = pl.ds(dd, 4, stride=PITCH)
            ref[k + it, 0, rows, :] = (a & jnp.uint32(0xFFFF)) | (b << 16)
            ref[k + it, 1, rows, :] = (a >> 16) | (b & jnp.uint32(0xFFFF0000))

    def wtile(t, h, it=0):
        start = (h // 2 % 4) * PITCH
        ref, k = where[4 * t + h // 8]
        return pltpu.bitcast(ref[k + it, h % 2, start:start + D // 2, :], bf16)

    def prepass(h, m, mb, it=0):
        lhs = pltpu.bitcast(xnb[mb * (m // 2):(mb + 1) * (m // 2), :], bf16)
        qkvb[h + 8 * it, mb * m:(mb + 1) * m, :] = jnp.dot(
            lhs, wtile(h // H, h % H, it), preferred_element_type=f32)

    def vfill(g, i):
        r0 = g * 16 if isinstance(g, int) else pl.multiple_of(g * 16, 16)
        lhs = pltpu.bitcast(xnb[pl.ds(r0, 16), :], bf16)
        vnext[i] = jnp.dot(lhs, wtile(2, H - NF + i), preferred_element_type=f32)

    route = {}

    def top_c():
        r = _rb(jnp.concatenate(scores, axis=1)) + 0.0
        tok = (lax.broadcasted_iota(jnp.int32, (8, 256), 1) * 8
               + lax.broadcasted_iota(jnp.int32, (8, 256), 0))
        bits = lax.shift_right_logical(pltpu.bitcast(r, jnp.int32), 16)
        rank = jnp.where(bits >= 0x8000, 0xFFFF - bits, bits + 0x8000)
        rank = jnp.where(r == r, rank, 0)
        key = pltpu.bitcast(rank * 2048 + (S - 1 - tok) + KEY0, f32)
        row16 = lax.broadcasted_iota(jnp.int32, (16, 128), 0)
        sel_ref[8:16, :] = jnp.zeros((8, D), f32)
        picked = jnp.full((16, 128), KEY0 + 0x8000 * 2048, jnp.int32)
        idxs = []
        for j in range(C):
            best = jnp.max(key, keepdims=True)
            key = jnp.where(key == best, 0.0, key)
            code = pltpu.bitcast(jnp.broadcast_to(best, (16, 128)), jnp.int32)
            picked = jnp.where(row16 == j, code, picked)
            t = (S - 1) - ((code[0, 0] - KEY0) & (S - 1))
            idx = (jnp.clip(t >> 5, 0, NSEG - 1), jnp.clip((t >> 3) & 3, 0, 3), jnp.clip(t & 7, 0, 7))
            idxs.append(idx)
            sel_ref[j:j + 1, :] = xb32[idx[0], idx[1], pl.ds(idx[2], 1), :]
        rank = lax.shift_right_logical(picked - KEY0, 11)
        bits = jnp.where(rank >= 0x8000, rank - 0x8000, 0xFFFF - rank)
        route['idx'] = idxs
        route['gate'] = jax.nn.sigmoid(pltpu.bitcast(bits << 16, f32))

    def ffn_gate(n):
        cols = slice(128 * n, min(128 * (n + 1), F))
        hg = lax.dot_general(sel_ref[0:16, :].astype(bf16), wg[cols, :], NT,
                             preferred_element_type=f32)
        route['g', n] = hg * jax.nn.sigmoid(hg)

    def ffn_up(n):
        cols = slice(128 * n, min(128 * (n + 1), F))
        hu = lax.dot_general(sel_ref[0:16, :].astype(bf16), wu[cols, :], NT,
                             preferred_element_type=f32)
        hh_ref[:, cols] = route['g', n] * hu

    def ffn_down(n, k0):
        cols = slice(128 * n, 128 * (n + 1))
        ks = slice(128 * k0, min(128 * (k0 + FKC), F))
        y = jnp.dot(hh_ref[:, ks].astype(bf16), wd[ks, cols], preferred_element_type=f32)
        src = slice(16, 32) if k0 else slice(0, 16)
        sel_ref[16:32, cols] = sel_ref[src, cols] + y * route['gate']

    def ffn_scatter():
        for j in range(C):
            idx = route['idx'][j]
            xb32[idx[0], idx[1], pl.ds(idx[2], 1), :] = sel_ref[16 + j:17 + j, :]

    def pp(h0, h1, m=PPM, it=0):
        return [P(prepass, h, m, mb, it) for h in range(h0, h1) for mb in range(512 // m)]

    def rl(*cs, it=0):
        return [P(relayout, c, i, it) for c in cs for i in range(20)]

    def block(name, waits, units, side, early=0):
        with jax.named_scope("wait_" + name):
            for cp in waits:
                cp.wait()
        with jax.named_scope("blk_" + name):
            if PRE:
                _interleave(units, side, early)

    block("lnb", [], layernorm(0, 0, NSEG // LNB, LNB, (0, 1, 2, 3), True), [])
    block("rl0", cp_w0[:1], rl(0)[:16], [])
    ffn = ([P(f, n) for n in range(14) for f in (ffn_gate, ffn_up)]
           + [P(ffn_down, n, k0) for k0 in range(0, 14, FKC) for n in range(KT)]
           + [ffn_scatter])

    def seq(*parts):
        return [lambda: [_interleave(*p) for p in parts]]

    if PLAN == 1:
        block("0", cp_w0[1:], rl(0)[16:] + pp(0, 4), [])
        block("1", cp_w[1:2], pp(4, 8), rl(1, it=zero if '1' in ONCE else 0), 1)

        def pre_body(it, carry):
            w_copy(it + 2, wq_hbm.at[:, pl.ds(0, 8), :]).wait()

            @pl.when((it & 1) == 1)
            def _():
                x_copy((it + 1) >> 1).wait()

            scores[:] = carry
            if PRE:
                ln = layernorm((it + 1) >> 1, ((it + 1) & 1) * 32, 32 // LNA, LNA, LNA_LAG, False)
                _interleave(pp(8, 16, PPML, it=it), _merge(rl(2, it=jnp.minimum(it, 6) if OPW else it), ln), EARLY)
            return tuple(scores)

        with jax.named_scope("blk_loop"):
            scores[:] = lax.fori_loop(0, 7, pre_body, tuple(scores))
        block("6", cp_w[9:12], pp(64, 72), [top_c] + rl(9, 10, 11, it=zero if '6' in ONCE else 0), 1)
        block("7", cp_ffn, pp(72, 3 * H - NF, PPM7),
              ffn + [P(vfill, 0, i) for i in range(NF)])
    else:
        block("0", cp_w0[1:], rl(0)[16:] + pp(0, H0), [])
        block("1", cp_w[1:2], seq((pp(H0, 8), rl(1, it=zero), 1), (pp(8, H1), [])), [])
        block("2", cp_w[2:4], seq((pp(H1, 16), rl(2, it=zero), 1),
                                  (pp(16, 24), rl(3, it=zero), 2)), [])

        def pre_body(it, carry):
            w_copy(2 * it + 4, wq_hbm.at[:, pl.ds(0, 8), :]).wait()
            w_copy(2 * it + 5, wq_hbm.at[:, pl.ds(0, 8), :]).wait()
            x_copy(it + 1).wait()
            if PLAN == 3:
                @pl.when(it > 0)
                def _():
                    w_copy(it + 9, wq_hbm.at[:, pl.ds(0, 8), :]).wait()
            scores[:] = carry
            if PRE:
                for half in range(2):
                    ln = layernorm(it + 1, 32 * half, 32 // LNA, LNA, LNA_LAG, False)
                    rls = rl(4 + half, it=2 * jnp.minimum(it, 2))
                    if PLAN == 3:
                        extra = rl(0, it=jnp.where(it > 0, it + 9, 0))
                        rls = _merge(rls, extra[10 * half:10 * half + 10])
                    _interleave(pp(24 + 8 * half, 32 + 8 * half, PPML, it=2 * it),
                                _merge(rls, ln), EARLY)
            return tuple(scores)

        with jax.named_scope("blk_loop"):
            scores[:] = lax.fori_loop(0, 3, pre_body, tuple(scores))
        vf = [P(vfill, 0, i) for i in range(NF)]
        block("7", (cp_w[10:12] if PLAN == 2 else []) + cp_ffn,
              seq((pp(72, 72 + TA, PPM7), [top_c] + (rl(10, 11, it=zero) if PLAN == 2 else []), 1),
                  (pp(72 + TA, 3 * H - NF, PPM7) + (vf if VFE else []), ffn + ([] if VFE else vf), E7)), [])
    block("wo", cp_wo + [cp_m0], [], [])

    def finish(s, lo, n, s_val):
        b = xb32[s, lo // 8:(lo + n) // 8].reshape(n, D)
        x = xbuf[s, lo // 8:(lo + n) // 8, :, 0:D].astype(f32).reshape(n, D)
        hb = 0.5 * b
        g = hb * jnp.tanh(hb) + hb
        obuf[s, lo // 8:(lo + n) // 8] = (x + s_val * g).reshape(n // 8, 8, D).astype(bf16)

    keep, fill = _masks()
    c80 = lax.broadcasted_iota(jnp.int32, (8, 80), 1)
    r80 = lax.broadcasted_iota(jnp.int32, (8, 80), 0)
    is_h0 = (c80 < 32) | ((c80 >= 64) & (c80 < 72))
    is_h1 = jnp.logical_not(is_h0)
    cj = c80 & 31
    cpos = jnp.where(c80 < 64, jnp.where(cj < 8, cj, cj + 8), 8 + (c80 & 7))
    causal = [None] + [cpos <= r80 + 8 + 8 * i for i in (1, 2, 3)] + [cpos <= r80 + 8]
    grp = [(0, 4), (1, 5), (2, 6), (3, 7), (8, 9)]
    scale = E ** -0.5

    def step(g, j, mem, vcur, held, fillers):
        s = 4 * g + j
        rows_b = pl.ds(pl.multiple_of(32 * g, 32) + 8 * j if GB else pl.multiple_of(8 * s, 8), 8)
        xa = [jnp.concatenate([xa32[XA0 + KT * jj + k, rows_b, :] for k in range(KT)], axis=1)
              for jj in (1, 2, 3)]
        lhs = jnp.concatenate([mem] + xa, axis=0).astype(bf16)
        nrow = 48 if j % 2 else 32
        st = {}

        def brows(t, h):
            if t == 2 and h >= H - NF:
                return vcur[h - (H - NF)][8 * j:8 * j + 8]
            return qkvb[t * H + h, rows_b, :]

        def proj(hp, t, par):
            st['y', par] = jnp.dot(lhs, wtile(t, 2 * hp + par), preferred_element_type=f32)
            if par == 1:
                st['qkv', hp, t] = jnp.concatenate(
                    [st['y', 0], st['y', 1], brows(t, 2 * hp), brows(t, 2 * hp + 1)],
                    axis=0).astype(bf16)

        def qk(hp):
            q, k = st['qkv', hp, 0], st['qkv', hp, 1]
            sc = lax.dot_general(q, k, NT, preferred_element_type=f32)
            if SM == 0:
                sc = jnp.where(keep, sc * scale, fill)
                p = jnp.exp(sc - jnp.max(sc, axis=-1, keepdims=True))
                l = jnp.sum(p, axis=-1, keepdims=True)
                st['p', hp] = (p * pl.reciprocal(l, approx=True)).astype(bf16)
                return
            rows = [None] * 10
            for i, gs in enumerate(grp):
                for g, hm in zip(gs, (is_h0, is_h1)):
                    sg = sc[8 * g:8 * g + 8] * scale
                    if causal[i] is not None:
                        sg = jnp.where(causal[i], sg, -1000000000.0)
                    sg = jnp.where(hm, sg, -jnp.inf)
                    e = jnp.exp(sg - jnp.max(sg, axis=-1, keepdims=True))
                    l = jnp.sum(e, axis=-1, keepdims=True)
                    rows[g] = e * pl.reciprocal(l, approx=True)
            st['p', hp] = jnp.concatenate(rows, axis=0).astype(bf16)

        def pv(hp):
            o = jnp.dot(st['p', hp], st['qkv', hp, 2], preferred_element_type=f32)
            for par in (0, 1):
                h = 2 * hp + par
                oa, ob = o[32 * par:32 * par + 32], o[64 + 8 * par:72 + 8 * par]
                if j % 2:
                    oa = jnp.concatenate([oa, held[h], ob], axis=0)
                else:
                    held[h] = ob
                st['o', h] = oa if CAT >= 3 else oa.astype(bf16)

        def oproj(n, h0, h1):
            a = jnp.concatenate([st['o', h] for h in range(h0, h1)], axis=1).astype(bf16)
            return jnp.dot(a, wo[n, h0 * 128:h1 * 128, :], preferred_element_type=f32)

        for t in range(NP + KT):
            for u in fillers.get(t, ()):
                u()
            for i in range(7):
                if POS[0] == i and 0 <= t - DQK < NP:
                    qk(t - DQK)
                if POS[1] == i and 0 <= t - DPV < NP:
                    pv(t - DPV)
                if i < 6:
                    which = 'qkv'.index(ORD[i // 2])
                    tt = t - DV if which == 2 else t
                    if 0 <= tt < NP:
                        proj(tt, which, i % 2)
                    if t >= NP and i == 0:
                        accs[t - NP, 0:nrow] = oproj(t - NP, 0, 2 * SPLIT)
        acc = jnp.concatenate([accs[n, 0:nrow] + oproj(n, 2 * SPLIT, H) for n in range(KT)],
                              axis=1)
        finish(s, 8, 24, acc[8:32])
        if j % 2:
            finish(s - 1, 0, 8, acc[32:40])
            finish(s, 0, 8, acc[40:48])
        return _rb(acc[0:8])

    def out_copy(g):
        segs = pl.ds(g * 4, 4)
        return pltpu.make_async_copy(obuf.at[segs], out_hbm.at[segs], osems.at[g])

    def group(g, mem):
        vcur = [vnext[i] for i in range(NF)]
        gn = jnp.minimum(g + 1, NG - 1)
        held = {}
        for j in range(4):
            fillers = {}
            for i, (jj, slot) in enumerate(FILL):
                if jj == j:
                    fillers.setdefault(slot, []).append(P(vfill, gn, i))
            mem = step(g, j, mem, vcur, held, fillers)
        out_copy(g).start()
        return mem

    with jax.named_scope("loop"):
        lax.fori_loop(0, NG, group, mem0_ref[0:8, :].astype(f32))
    with jax.named_scope("wait_out"):
        for g in range(NG):
            out_copy(g).wait()


@functools.partial(jax.jit, static_argnames=("A_seg_len",))
def pallas_recurrent_scan__memory_aug_recurrent_mem_tr__moe_arch_mod__prompt_kernel(
    A_x: jax.Array,
    A_mem0: jax.Array,
    A_Wq: jax.Array,
    A_Wk: jax.Array,
    A_Wv: jax.Array,
    A_Wo: jax.Array,
    A_seg_len,
    B_x: jax.Array,
    B_w_r: jax.Array,
    B_w_gate: jax.Array,
    B_w_up: jax.Array,
    B_w_down: jax.Array,
):
    del B_x
    assert A_seg_len == SEG
    assert A_x.shape == (1, S, D) and A_Wq.shape == (D, H, E) and B_w_gate.shape == (D, F)
    hbm = pl.BlockSpec(memory_space=pl.ANY)
    out = pl.pallas_call(
        _kernel,
        out_shape=jax.ShapeDtypeStruct((NSEG, 4, 8, D), bf16),
        in_specs=[hbm] * 10,
        out_specs=hbm,
        scratch_shapes=[
            pltpu.VMEM((NSEG, 4, 8, XW), bf16),
            pltpu.VMEM((1 if ALIAS else 4 * KT, NSEG * 8, E), f32),
            pltpu.VMEM((NSEG, 4, 8, D), f32),
            pltpu.VMEM((NSEG * 4, D), u32),
            pltpu.VMEM((32, D), f32),
            pltpu.VMEM((16, F), f32),
            pltpu.VMEM((NCH, D, 8, E), bf16),
            pltpu.VMEM((KT, H * E, 128), bf16),
            pltpu.VMEM((3 * H + 4 * KT + 1, NSEG * 8, E), f32),
            pltpu.VMEM((NF, 32, E), f32),
            pltpu.VMEM((F, D), bf16),
            pltpu.VMEM((F, D), bf16),
            pltpu.VMEM((F, D), bf16),
            pltpu.VMEM((NSEG, 4, 8, D), bf16),
            pltpu.VMEM((KT, 64, 128), f32),
            pltpu.VMEM((64, D), bf16),
            pltpu.SemaphoreType.DMA((29,)),
            pltpu.SemaphoreType.DMA((NG,)),
        ] + [pltpu.VMEM((len(g), 2, 4 * PITCH, E), u32) for g in WGR]
        + [pltpu.VMEM((D,), bf16)],
        compiler_params=pltpu.CompilerParams(
            vmem_limit_bytes=120 * 1024 * 1024,
            disable_bounds_checks=True, disable_semaphore_checks=True),
    )(A_x.reshape(NSEG, 4, 8, D), A_mem0.reshape(M, D), A_Wq, A_Wk, A_Wv, A_Wo.reshape(H * E, D),
      B_w_r, B_w_gate.T, B_w_up.T, B_w_down)
    return out.reshape(1, S, D)
```

```python
import functools

import jax
import jax.numpy as jnp
from jax import lax
import jax.experimental.pallas as pl
import jax.experimental.pallas.tpu as pltpu

bf16 = jnp.bfloat16
f32 = jnp.float32
u32 = jnp.uint32
P = functools.partial

S, D, H, E = 2048, 640, 32, 128
M, SEG = 8, 32
NSEG = S // SEG
NG = NSEG // 4
NP = H // 2
F, C = 1728, 8
KT = D // 128
NCH = 12
PITCH = 328
XA0 = 3 * H
PIN = XA0 + 4 * KT
EPS_BF16 = 1.0013580322265625e-05
KEY0 = 0x3F800000
NT = (((1,), (1,)), ((), ()))

DQK, DV, DPV = 1, 2, 4
SPLIT = (22, 20)
FILL = (1, 1, 2, 2, 3, 3)
NF = len(FILL)
KS = 3
FKC = 5


def _rb(v):
    return v.astype(bf16).astype(f32)


def _merge(a, b):
    keyed = [((i + 0.5) / len(a), 0, t) for i, t in enumerate(a)]
    keyed += [((i + 0.5) / len(b), 1, t) for i, t in enumerate(b)]
    return [t for _, _, t in sorted(keyed, key=lambda e: e[:2])]


def _emit(units, side=(), early=0):
    done = 0
    for i, unit in enumerate(units):
        unit()
        want = min(len(side), (len(side) * (i + 1)) // (len(units) - early))
        for task in side[done:want]:
            task()
        done = want


def _kernel(x_hbm, mem0_hbm, wq_hbm, wk_hbm, wv_hbm, wo_hbm, wr_hbm, wg_hbm, wu_hbm, wd_hbm,
            out_hbm,
            xbuf, xb32, xnb, sel_ref, hh_ref, wraw, wo, act, vnext,
            wg, wu, wd, obuf, accs, mem0_ref, sems, osems, wqkv, wr_ref):
    w_hbm = (wq_hbm, wk_hbm, wv_hbm)

    def x_copy(j):
        return pltpu.make_async_copy(x_hbm.at[:, j], xbuf.at[:, j, :, pl.ds(0, D)],
                                     sems.at[25 + j])

    def w_copy(c, src):
        return pltpu.make_async_copy(src, wraw.at[c], sems.at[1 + c])

    def w_wait(c):
        w_copy(c, wq_hbm.at[:, pl.ds(0, 8), :]).wait()

    cp_x = [None] + [x_copy(j) for j in range(1, 4)]
    cp_w = [None] + [w_copy(c, w_hbm[c // 4].at[:, pl.ds(8 * (c % 4), 8), :])
                     for c in range(1, NCH)]
    cp_w0 = [pltpu.make_async_copy(wq_hbm.at[pl.ds(lo, hi - lo), pl.ds(0, 8), :],
                                   wraw.at[0, pl.ds(lo, hi - lo)], sems.at[sem])
             for sem, lo, hi in ((13, 0, 128 * KS - 128), (14, 128 * KS - 128, 128 * KS),
                                 (0, 128 * KS, D))]
    cp_x0 = [pltpu.make_async_copy(x_hbm.at[pl.ds(32 * i, 32), 0],
                                   xbuf.at[pl.ds(32 * i, 32), 0, :, pl.ds(0, D)], sems.at[sem])
             for i, sem in enumerate((25, 1))]
    cp_ffn = [pltpu.make_async_copy(src, dst, sems.at[15 + i])
              for i, (src, dst) in enumerate(((wg_hbm, wg), (wu_hbm, wu), (wd_hbm, wd)))]
    cp_wo = [pltpu.make_async_copy(wo_hbm.at[:, pl.ds(128 * n, 128)], wo.at[n], sems.at[18 + n])
             for n in range(KT)]
    cp_wr = pltpu.make_async_copy(wr_hbm, wr_ref, sems.at[23])
    cp_m0 = pltpu.make_async_copy(mem0_hbm, mem0_ref.at[pl.ds(0, 8)], sems.at[24])
    for cp in ([cp_x0[0], cp_wr] + cp_w0 + [cp_x0[1]] + cp_w[1:6] + [cp_x[1]] + cp_w[6:8]
               + [cp_x[2], cp_w[10]] + cp_w[8:10] + [cp_x[3], cp_w[11]] + cp_ffn + cp_wo
               + [cp_m0]):
        cp.start()
    zero = lax.fori_loop(0, 2, lambda i, c: (c + i) >> 1, 0)
    cp_x0[0].wait()
    cp_wr.wait()

    wr = wr_ref[...].astype(f32).reshape(1, D)
    lane = lax.broadcasted_iota(jnp.int32, (8, 128), 1)
    scores = [jnp.zeros((8, 128), f32), jnp.zeros((8, 128), f32)]

    def layernorm(j, s0, nb, lag, pin):
        st = {}
        n = 32 // nb
        lane_j = lane - j

        def load(i):
            return xbuf[pl.ds(s0 + nb * i, nb), j, :, 0:D].astype(f32).reshape(8 * nb, D)

        def mean(i):
            st['mu', i] = jnp.mean(load(i), axis=-1, keepdims=True)

        def var(i):
            xc = load(i) - st['mu', i]
            st['var', i] = jnp.mean(xc * xc, axis=-1, keepdims=True)

        def norm(i):
            lo, hi = s0 + nb * i, s0 + nb * (i + 1)
            v = _rb(_rb(st['var', i]) + EPS_BF16)
            den = _rb(v * lax.rsqrt(v))
            inv = pl.reciprocal(den, approx=True)
            inv = inv * (2.0 - den * inv)
            xn = (load(i) - _rb(st['mu', i])) * inv
            xb32[pl.ds(lo, nb), j] = xn.reshape(nb, 8, D)
            if isinstance(j, int):
                xnb[4 * lo:4 * hi, :] = pltpu.bitcast(xn.astype(bf16), u32)
            else:
                for k in range(KT):
                    act[XA0 + KT * j + k, 8 * lo:8 * hi, :] = xn[:, 128 * k:128 * (k + 1)]
            st['r', i] = jnp.sum(xn * wr, axis=-1, keepdims=True)

        def score(i):
            v = s0 // 32
            for k in range(nb):
                scores[v] = jnp.where(lane_j == 4 * (nb * i + k), st['r', i][8 * k:8 * k + 8],
                                      scores[v])
            if pin is not None:
                act[pin, 0:8, :] = scores[v]

        def stage(t):
            for d, fn in zip(lag, (mean, var, norm, score)):
                if 0 <= t - d < n:
                    fn(t - d)

        return [P(stage, t) for t in range(n + lag[-1])]

    def relayout(c, i):
        for dd in range(16 * i, 16 * i + 16):
            a = pltpu.bitcast(wraw[c, 2 * dd], u32)
            b = pltpu.bitcast(wraw[c, 2 * dd + 1], u32)
            rows = pl.ds(dd, 4, stride=PITCH)
            wqkv[c, 0, rows, :] = (a & jnp.uint32(0xFFFF)) | (b << 16)
            wqkv[c, 1, rows, :] = (a >> 16) | (b & jnp.uint32(0xFFFF0000))

    def wtile(h, dc=0, k0=0, k1=KT):
        start = (h // 2 % 4) * PITCH
        w = wqkv[h // 8 + dc, h % 2, start + 64 * k0:start + 64 * k1, :]
        return pltpu.bitcast(w, bf16)

    def prepass(h, mb, dc=0, k0=0, k1=KT):
        rows = slice(128 * mb, 128 * (mb + 1))
        lhs = pltpu.bitcast(xnb[64 * mb:64 * (mb + 1), 128 * k0:128 * k1], bf16)
        y = jnp.dot(lhs, wtile(h, dc, k0, k1), preferred_element_type=f32)
        act[h + 8 * dc, rows, :] = y if k0 == 0 else act[h + 8 * dc, rows, :] + y

    def vfill(g, i):
        r0 = g * 16 if isinstance(g, int) else pl.multiple_of(g * 16, 16)
        lhs = pltpu.bitcast(xnb[pl.ds(r0, 16), :], bf16)
        vnext[i] = jnp.dot(lhs, wtile(3 * H - NF + i), preferred_element_type=f32)

    def pp(h0, h1, mbs=range(4), **kw):
        return [P(prepass, h, mb, **kw) for h in range(h0, h1) for mb in mbs]

    def rl(c):
        return [P(relayout, c, i) for i in range(20)]

    route = {}

    def top_c():
        r = _rb(jnp.concatenate(scores, axis=1))
        tok = (lax.broadcasted_iota(jnp.int32, (8, 256), 1) * 8
               + lax.broadcasted_iota(jnp.int32, (8, 256), 0))
        bits = lax.shift_right_logical(pltpu.bitcast(r, jnp.int32), 16)
        rank = jnp.where(bits >= 0x8000, 0x10000 - bits, bits + 0x8000)
        rank = jnp.where(r == r, rank, 0)
        key = pltpu.bitcast(rank * 2048 + (S - 1 - tok) + KEY0, f32)
        row16 = lax.broadcasted_iota(jnp.int32, (16, 128), 0)
        sel_ref[8:16, :] = jnp.zeros((8, D), f32)
        picked = jnp.full((16, 128), KEY0 + 0x8000 * 2048, jnp.int32)
        idxs = []
        for j in range(C):
            best = jnp.max(key, keepdims=True)
            key = jnp.where(key == best, 0.0, key)
            code = pltpu.bitcast(jnp.broadcast_to(best, (16, 128)), jnp.int32)
            picked = jnp.where(row16 == j, code, picked)
            t = (S - 1) - ((code[0, 0] - KEY0) & (S - 1))
            idx = (jnp.clip(t >> 5, 0, NSEG - 1), jnp.clip((t >> 3) & 3, 0, 3),
                   jnp.clip(t & 7, 0, 7))
            idxs.append(idx)
            sel_ref[j:j + 1, :] = xb32[idx[0], idx[1], pl.ds(idx[2], 1), :]
        rank = lax.shift_right_logical(picked - KEY0, 11)
        bits = jnp.where(rank >= 0x8000, rank - 0x8000, 0x10000 - rank)
        route['idx'] = idxs
        route['gate'] = jax.nn.sigmoid(pltpu.bitcast(bits << 16, f32))

    def ffn_gate(n):
        cols = slice(128 * n, min(128 * (n + 1), F))
        hg = lax.dot_general(sel_ref[0:16, :].astype(bf16), wg[cols, :], NT,
                             preferred_element_type=f32)
        route['g', n] = hg * jax.nn.sigmoid(hg)

    def ffn_up(n):
        cols = slice(128 * n, min(128 * (n + 1), F))
        hu = lax.dot_general(sel_ref[0:16, :].astype(bf16), wu[cols, :], NT,
                             preferred_element_type=f32)
        hh_ref[:, cols] = route['g', n] * hu

    def ffn_down(n, k0):
        cols = slice(128 * n, 128 * (n + 1))
        ks = slice(128 * k0, min(128 * (k0 + FKC), F))
        y = jnp.dot(hh_ref[:, ks].astype(bf16), wd[ks, cols], preferred_element_type=f32)
        src = slice(16, 32) if k0 else slice(0, 16)
        sel_ref[16:32, cols] = sel_ref[src, cols] + y * route['gate']

    def ffn_scatter():
        for j in range(C):
            idx = route['idx'][j]
            xb32[idx[0], idx[1], pl.ds(idx[2], 1), :] = sel_ref[16 + j:17 + j, :]

    _emit(layernorm(0, 0, 8, (0, 1, 2, 3), None))
    cp_w0[0].wait()
    _emit(rl(0)[:4 * KS - 4])
    cp_w0[1].wait()
    _emit(rl(0)[4 * KS - 4:4 * KS] + pp(0, 6, (0, 1), k1=KS))
    cp_w0[2].wait()
    cp_x0[1].wait()
    ln1 = layernorm(0, 32, 4, (0, 1, 2, 3), PIN + zero)
    _emit(pp(6, 8, (0, 1), k1=KS), _merge(rl(zero)[4 * KS:], ln1[:3]), 1)
    _emit(pp(0, 8, (0, 1), k0=KS), ln1[3:], 2)
    _emit(pp(0, 4, (2, 3)))
    cp_w[1].wait()
    _emit(pp(4, 8, (2, 3)), rl(1 + zero), 1)
    _emit(pp(8, 14))
    cp_w[2].wait()
    cp_w[3].wait()
    _emit(pp(14, 16), rl(2 + zero), 1)
    _emit(pp(16, 24), rl(3 + zero), 2)

    def pre_body(it, carry):
        w_wait(2 * it + 4)
        w_wait(2 * it + 5)
        x_copy(it + 1).wait()

        @pl.when(it > 0)
        def _():
            w_wait(it + 9)

        scores[:] = carry
        for half in range(2):
            ln = layernorm(it + 1, 32 * half, 2, (0, 1, 2, 4), PIN)
            rls = _merge(rl(4 + half + 2 * jnp.minimum(it, 2)),
                         rl(jnp.where(it > 0, it + 9, 0))[10 * half:10 * half + 10])
            _emit(pp(24 + 8 * half, 32 + 8 * half, dc=2 * it), _merge(rls, ln), 2)
        return tuple(scores)

    scores[:] = lax.fori_loop(0, 3, pre_body, tuple(scores))
    for cp in cp_ffn:
        cp.wait()
    _emit(pp(72, 75), [top_c], 1)
    _emit(pp(75, 3 * H - NF) + [P(vfill, 0, i) for i in range(NF)],
          [P(fn, n) for n in range(14) for fn in (ffn_gate, ffn_up)]
          + [P(ffn_down, n, k0) for k0 in range(0, 14, FKC) for n in range(KT)]
          + [ffn_scatter], 9)
    for cp in cp_wo + [cp_m0]:
        cp.wait()

    def finish(s, lo, n, s_val):
        b = xb32[s, lo // 8:(lo + n) // 8].reshape(n, D)
        x = xbuf[s, lo // 8:(lo + n) // 8, :, 0:D].astype(f32).reshape(n, D)
        hb = 0.5 * b
        g = hb * jnp.tanh(hb) + hb
        obuf[s, lo // 8:(lo + n) // 8] = (x + s_val * g).reshape(n // 8, 8, D).astype(bf16)

    col = lax.broadcasted_iota(jnp.int32, (8, 80), 1)
    row = lax.broadcasted_iota(jnp.int32, (8, 80), 0)
    is_h0 = (col < 32) | ((col >= 64) & (col < 72))
    own = (is_h0, jnp.logical_not(is_h0))
    cj = col & 31
    cpos = jnp.where(col < 64, jnp.where(cj < 8, cj, cj + 8), 8 + (col & 7))
    groups = ((0, 4), (1, 5), (2, 6), (3, 7), (8, 9))
    causal = [None] + [cpos <= row + 8 + 8 * i for i in (1, 2, 3)] + [cpos <= row + 8]
    scale = E ** -0.5

    def step(g, j, mem, vcur, held, fillers):
        s = 4 * g + j
        rows_b = pl.ds(pl.multiple_of(32 * g, 32) + 8 * j, 8)
        xa = [jnp.concatenate([act[XA0 + KT * jj + k, rows_b, :] for k in range(KT)], axis=1)
              for jj in (1, 2, 3)]
        lhs = jnp.concatenate([mem] + xa, axis=0).astype(bf16)
        nrow = 48 if j % 2 else 32
        split = SPLIT[j % 2]
        st = {}

        def brows(h):
            if h >= 3 * H - NF:
                return vcur[h - (3 * H - NF)][8 * j:8 * j + 8]
            return act[h, rows_b, :]

        def proj(t, hp, par):
            if not 0 <= hp < NP:
                return
            h = t * H + 2 * hp
            st['y', par] = jnp.dot(lhs, wtile(h + par), preferred_element_type=f32)
            if par == 1:
                st['qkv', t, hp] = jnp.concatenate(
                    [st['y', 0], st['y', 1], brows(h), brows(h + 1)], axis=0).astype(bf16)

        def qk(hp):
            sc = lax.dot_general(st['qkv', 0, hp], st['qkv', 1, hp], NT,
                                 preferred_element_type=f32)
            rows = [None] * 10
            for gs, cm in zip(groups, causal):
                for r, hm in zip(gs, own):
                    sg = sc[8 * r:8 * r + 8] * scale
                    if cm is not None:
                        sg = jnp.where(cm, sg, -1000000000.0)
                    sg = jnp.where(hm, sg, -jnp.inf)
                    e = jnp.exp(sg - jnp.max(sg, axis=-1, keepdims=True))
                    l = jnp.sum(e, axis=-1, keepdims=True)
                    rows[r] = e * pl.reciprocal(l, approx=True)
            st['p', hp] = jnp.concatenate(rows, axis=0).astype(bf16)

        def pv(hp):
            o = jnp.dot(st['p', hp], st['qkv', 2, hp], preferred_element_type=f32)
            for par in (0, 1):
                h = 2 * hp + par
                oa, ob = o[32 * par:32 * par + 32], o[64 + 8 * par:72 + 8 * par]
                if j % 2:
                    oa = jnp.concatenate([oa, held[h], ob], axis=0)
                else:
                    held[h] = ob
                st['o', h] = oa

        def oproj(n, h0, h1):
            a = jnp.concatenate([st['o', h] for h in range(h0, h1)], axis=1).astype(bf16)
            return jnp.dot(a, wo[n, h0 * 128:h1 * 128, :], preferred_element_type=f32)

        for u in fillers:
            u()
        for t in range(NP + KT):
            proj(1, t, 0)
            proj(1, t, 1)
            proj(0, t, 0)
            if t >= NP:
                accs[t - NP, 0:nrow] = oproj(t - NP, 0, split)
            proj(0, t, 1)
            if 0 <= t - DQK < NP:
                qk(t - DQK)
            if 0 <= t - DPV < NP:
                pv(t - DPV)
            proj(2, t - DV, 0)
            proj(2, t - DV, 1)
        acc = jnp.concatenate([accs[n, 0:nrow] + oproj(n, split, H) for n in range(KT)], axis=1)
        finish(s, 8, 24, acc[8:32])
        if j % 2:
            finish(s - 1, 0, 8, acc[32:40])
            finish(s, 0, 8, acc[40:48])
        return _rb(acc[0:8])

    def out_copy(g):
        segs = pl.ds(g * 4, 4)
        return pltpu.make_async_copy(obuf.at[segs], out_hbm.at[segs], osems.at[g])

    def group(g, mem):
        vcur = [vnext[i] for i in range(NF)]
        gn = jnp.minimum(g + 1, NG - 1)
        held = {}
        for j in range(4):
            fillers = [P(vfill, gn, i) for i in range(NF) if FILL[i] == j]
            mem = step(g, j, mem, vcur, held, fillers)
        out_copy(g).start()
        return mem

    lax.fori_loop(0, NG, group, mem0_ref[0:8, :].astype(f32))
    for g in range(NG):
        out_copy(g).wait()


@functools.partial(jax.jit, static_argnames=("A_seg_len",))
def pallas_recurrent_scan__memory_aug_recurrent_mem_tr__moe_arch_mod__prompt_kernel(
    A_x: jax.Array,
    A_mem0: jax.Array,
    A_Wq: jax.Array,
    A_Wk: jax.Array,
    A_Wv: jax.Array,
    A_Wo: jax.Array,
    A_seg_len,
    B_x: jax.Array,
    B_w_r: jax.Array,
    B_w_gate: jax.Array,
    B_w_up: jax.Array,
    B_w_down: jax.Array,
):
    del B_x
    assert A_seg_len == SEG
    assert A_x.shape == (1, S, D) and A_Wq.shape == (D, H, E) and B_w_gate.shape == (D, F)
    hbm = pl.BlockSpec(memory_space=pl.ANY)
    out = pl.pallas_call(
        _kernel,
        out_shape=jax.ShapeDtypeStruct((NSEG, 4, 8, D), bf16),
        in_specs=[hbm] * 10,
        out_specs=hbm,
        scratch_shapes=[
            pltpu.VMEM((NSEG, 4, 8, 1024), bf16),
            pltpu.VMEM((NSEG, 4, 8, D), f32),
            pltpu.VMEM((NSEG * 4, D), u32),
            pltpu.VMEM((32, D), f32),
            pltpu.VMEM((16, F), f32),
            pltpu.VMEM((NCH, D, 8, E), bf16),
            pltpu.VMEM((KT, H * E, 128), bf16),
            pltpu.VMEM((PIN + 1, NSEG * 8, E), f32),
            pltpu.VMEM((NF, 32, E), f32),
            pltpu.VMEM((F, D), bf16),
            pltpu.VMEM((F, D), bf16),
            pltpu.VMEM((F, D), bf16),
            pltpu.VMEM((NSEG, 4, 8, D), bf16),
            pltpu.VMEM((KT, 64, 128), f32),
            pltpu.VMEM((64, D), bf16),
            pltpu.SemaphoreType.DMA((29,)),
            pltpu.SemaphoreType.DMA((NG,)),
            pltpu.VMEM((NCH, 2, 4 * PITCH, E), u32),
            pltpu.VMEM((D,), bf16),
        ],
        compiler_params=pltpu.CompilerParams(
            vmem_limit_bytes=120 * 1024 * 1024,
            disable_bounds_checks=True, disable_semaphore_checks=True),
    )(A_x.reshape(NSEG, 4, 8, D), A_mem0.reshape(M, D), A_Wq, A_Wk, A_Wv, A_Wo.reshape(H * E, D),
      B_w_r, B_w_gate.T, B_w_up.T, B_w_down)
    return out.reshape(1, S, D)
```

```python
import functools

import jax
import jax.numpy as jnp
from jax import lax
import jax.experimental.pallas as pl
import jax.experimental.pallas.tpu as pltpu

bf16 = jnp.bfloat16
f32 = jnp.float32
u32 = jnp.uint32
P = functools.partial

S, D, H, E = 2048, 640, 32, 128
M, SEG = 8, 32
NSEG = S // SEG
NG = NSEG // 4
NP = H // 2
F, C = 1728, 8
KT = D // 128
NCH = 12
PITCH = 328
XA0 = 3 * H
PIN = XA0 + 4 * KT
EPS_BF16 = 1.0013580322265625e-05
KEY0 = 0x3F800000
NT = (((1,), (1,)), ((), ()))

STEPS = (('kqv', 3, 4, 2, 3, 22, 0),
         ('kqv', 6, 5, 2, 3, 26, 2),
         ('qkv', 5, 5, 1, 3, 24, 2),
         ('kqv', 4, 3, 1, 3, 22, 0))
FILL = (1, 1, 2, 2, 3, 3)
NF = len(FILL)
KS = 3
FKC = 5


def _rb(v):
    return v.astype(bf16).astype(f32)


def _merge(a, b):
    keyed = [((i + 0.5) / len(a), 0, t) for i, t in enumerate(a)]
    keyed += [((i + 0.5) / len(b), 1, t) for i, t in enumerate(b)]
    return [t for _, _, t in sorted(keyed, key=lambda e: e[:2])]


def _emit(units, side=(), early=0):
    done = 0
    for i, unit in enumerate(units):
        unit()
        want = min(len(side), (len(side) * (i + 1)) // (len(units) - early))
        for task in side[done:want]:
            task()
        done = want


def _kernel(x_hbm, mem0_hbm, wq_hbm, wk_hbm, wv_hbm, wo_hbm, wr_hbm, wg_hbm, wu_hbm, wd_hbm,
            out_hbm,
            xbuf, xb32, xnb, sel_ref, hh_ref, wraw, wo, act, vnext,
            wg, wu, wd, obuf, accs, mem0_ref, sems, osems, wqkv, wr_ref):
    w_hbm = (wq_hbm, wk_hbm, wv_hbm)

    def x_copy(j):
        return pltpu.make_async_copy(x_hbm.at[:, j], xbuf.at[:, j, :, pl.ds(0, D)],
                                     sems.at[25 + j])

    def w_copy(c, src):
        return pltpu.make_async_copy(src, wraw.at[c], sems.at[1 + c])

    def w_wait(c):
        w_copy(c, wq_hbm.at[:, pl.ds(0, 8), :]).wait()

    cp_x = [None] + [x_copy(j) for j in range(1, 4)]
    cp_w = [None] + [w_copy(c, w_hbm[c // 4].at[:, pl.ds(8 * (c % 4), 8), :])
                     for c in range(1, NCH)]
    cp_w0 = [pltpu.make_async_copy(wq_hbm.at[pl.ds(lo, hi - lo), pl.ds(0, 8), :],
                                   wraw.at[0, pl.ds(lo, hi - lo)], sems.at[sem])
             for sem, lo, hi in ((13, 0, 128 * KS - 128), (14, 128 * KS - 128, 128 * KS),
                                 (0, 128 * KS, D))]
    cp_x0 = [pltpu.make_async_copy(x_hbm.at[pl.ds(32 * i, 32), 0],
                                   xbuf.at[pl.ds(32 * i, 32), 0, :, pl.ds(0, D)], sems.at[sem])
             for i, sem in enumerate((25, 1))]
    cp_ffn = [pltpu.make_async_copy(src, dst, sems.at[15 + i])
              for i, (src, dst) in enumerate(((wg_hbm, wg), (wu_hbm, wu), (wd_hbm, wd)))]
    cp_wo = [pltpu.make_async_copy(wo_hbm.at[:, pl.ds(128 * n, 128)], wo.at[n], sems.at[18 + n])
             for n in range(KT)]
    cp_wr = pltpu.make_async_copy(wr_hbm, wr_ref, sems.at[23])
    cp_m0 = pltpu.make_async_copy(mem0_hbm, mem0_ref.at[pl.ds(0, 8)], sems.at[24])
    for cp in ([cp_wr, cp_x0[0]] + cp_w0 + [cp_x0[1]] + cp_w[1:6] + [cp_x[1]] + cp_w[6:8]
               + [cp_x[2], cp_w[10]] + cp_w[8:10] + [cp_x[3], cp_w[11]] + cp_ffn + cp_wo
               + [cp_m0]):
        cp.start()
    zero = lax.fori_loop(0, 2, lambda i, c: (c + i) >> 1, 0)

    def out_copy(g):
        segs = pl.ds(g * 2, 2)
        return pltpu.make_async_copy(obuf.at[segs], out_hbm.at[segs], osems.at[g])

    def everything(_, carry):
        cp_x0[0].wait()
        cp_wr.wait()

        wr = wr_ref[...].astype(f32).reshape(1, D)
        lane = lax.broadcasted_iota(jnp.int32, (8, 128), 1)
        scores = [jnp.zeros((8, 128), f32), jnp.zeros((8, 128), f32)]

        def layernorm(j, s0, nb, lag, pin):
            st = {}
            n = 32 // nb
            lane_j = lane - j

            def load(i):
                return xbuf[pl.ds(s0 + nb * i, nb), j, :, 0:D].astype(f32).reshape(8 * nb, D)

            def mean(i):
                st['mu', i] = jnp.mean(load(i), axis=-1, keepdims=True)

            def var(i):
                xc = load(i) - st['mu', i]
                st['var', i] = jnp.mean(xc * xc, axis=-1, keepdims=True)

            def norm(i):
                lo, hi = s0 + nb * i, s0 + nb * (i + 1)
                v = _rb(_rb(st['var', i]) + EPS_BF16)
                den = _rb(v * lax.rsqrt(v))
                inv = pl.reciprocal(den, approx=True)
                inv = inv * (2.0 - den * inv)
                xn = (load(i) - _rb(st['mu', i])) * inv
                xb32[pl.ds(lo, nb), j] = xn.reshape(nb, 8, D)
                if isinstance(j, int):
                    xnb[4 * lo:4 * hi, :] = pltpu.bitcast(xn.astype(bf16), u32)
                else:
                    for k in range(KT):
                        act[XA0 + KT * j + k, 8 * lo:8 * hi, :] = xn[:, 128 * k:128 * (k + 1)]
                st['r', i] = jnp.sum(xn * wr, axis=-1, keepdims=True)

            def score(i):
                v = s0 // 32
                for k in range(nb):
                    scores[v] = jnp.where(lane_j == 4 * (nb * i + k), st['r', i][8 * k:8 * k + 8],
                                          scores[v])
                if pin is not None:
                    act[pin, 0:8, :] = scores[v]

            def stage(t):
                for d, fn in zip(lag, (mean, var, norm, score)):
                    if 0 <= t - d < n:
                        fn(t - d)

            return [P(stage, t) for t in range(n + lag[-1])]

        def relayout(c, i):
            for dd in range(16 * i, 16 * i + 16):
                a = pltpu.bitcast(wraw[c, 2 * dd], u32)
                b = pltpu.bitcast(wraw[c, 2 * dd + 1], u32)
                rows = pl.ds(dd, 4, stride=PITCH)
                wqkv[c, 0, rows, :] = (a & jnp.uint32(0xFFFF)) | (b << 16)
                wqkv[c, 1, rows, :] = (a >> 16) | (b & jnp.uint32(0xFFFF0000))

        def wtile(h, dc=0, k0=0, k1=KT):
            start = (h // 2 % 4) * PITCH
            w = wqkv[h // 8 + dc, h % 2, start + 64 * k0:start + 64 * k1, :]
            return pltpu.bitcast(w, bf16)

        def prepass(h, mb, dc=0, k0=0, k1=KT):
            rows = slice(128 * mb, 128 * (mb + 1))
            lhs = pltpu.bitcast(xnb[64 * mb:64 * (mb + 1), 128 * k0:128 * k1], bf16)
            y = jnp.dot(lhs, wtile(h, dc, k0, k1), preferred_element_type=f32)
            act[h + 8 * dc, rows, :] = y if k0 == 0 else act[h + 8 * dc, rows, :] + y

        def vfill(g, i):
            r0 = g * 16 if isinstance(g, int) else pl.multiple_of(g * 16, 16)
            lhs = pltpu.bitcast(xnb[pl.ds(r0, 16), :], bf16)
            vnext[i] = jnp.dot(lhs, wtile(3 * H - NF + i), preferred_element_type=f32)

        def pp(h0, h1, mbs=range(4), **kw):
            return [P(prepass, h, mb, **kw) for h in range(h0, h1) for mb in mbs]

        def rl(c):
            return [P(relayout, c, i) for i in range(20)]

        route = {}

        def top_c():
            r = _rb(jnp.concatenate(scores, axis=1))
            tok = (lax.broadcasted_iota(jnp.int32, (8, 256), 1) * 8
                   + lax.broadcasted_iota(jnp.int32, (8, 256), 0))
            bits = lax.shift_right_logical(pltpu.bitcast(r, jnp.int32), 16)
            rank = jnp.where(bits >= 0x8000, 0x10000 - bits, bits + 0x8000)
            rank = jnp.where(r == r, rank, 0)
            key = pltpu.bitcast(rank * 2048 + (S - 1 - tok) + KEY0, f32)
            row16 = lax.broadcasted_iota(jnp.int32, (16, 128), 0)
            sel_ref[8:16, :] = jnp.zeros((8, D), f32)
            picked = jnp.full((16, 128), KEY0 + 0x8000 * 2048, jnp.int32)
            idxs = []
            for j in range(C):
                best = jnp.max(key, keepdims=True)
                key = jnp.where(key == best, 0.0, key)
                code = pltpu.bitcast(jnp.broadcast_to(best, (16, 128)), jnp.int32)
                picked = jnp.where(row16 == j, code, picked)
                t = (S - 1) - ((code[0, 0] - KEY0) & (S - 1))
                idx = (jnp.clip(t >> 5, 0, NSEG - 1), jnp.clip((t >> 3) & 3, 0, 3),
                       jnp.clip(t & 7, 0, 7))
                idxs.append(idx)
                sel_ref[j:j + 1, :] = xb32[idx[0], idx[1], pl.ds(idx[2], 1), :]
            rank = lax.shift_right_logical(picked - KEY0, 11)
            bits = jnp.where(rank >= 0x8000, rank - 0x8000, 0x10000 - rank)
            route['idx'] = idxs
            route['gate'] = jax.nn.sigmoid(pltpu.bitcast(bits << 16, f32))

        def ffn_gate(n):
            cols = slice(128 * n, min(128 * (n + 1), F))
            hg = lax.dot_general(sel_ref[0:16, :].astype(bf16), wg[cols, :], NT,
                                 preferred_element_type=f32)
            route['g', n] = hg * jax.nn.sigmoid(hg)

        def ffn_up(n):
            cols = slice(128 * n, min(128 * (n + 1), F))
            hu = lax.dot_general(sel_ref[0:16, :].astype(bf16), wu[cols, :], NT,
                                 preferred_element_type=f32)
            hh_ref[:, cols] = route['g', n] * hu

        def ffn_down(n, k0):
            cols = slice(128 * n, 128 * (n + 1))
            ks = slice(128 * k0, min(128 * (k0 + FKC), F))
            y = jnp.dot(hh_ref[:, ks].astype(bf16), wd[ks, cols], preferred_element_type=f32)
            src = slice(16, 32) if k0 else slice(0, 16)
            sel_ref[16:32, cols] = sel_ref[src, cols] + y * route['gate']

        def ffn_scatter():
            for j in range(C):
                idx = route['idx'][j]
                xb32[idx[0], idx[1], pl.ds(idx[2], 1), :] = sel_ref[16 + j:17 + j, :]

        _emit(layernorm(0, 0, 8, (0, 1, 2, 3), None))
        cp_w0[0].wait()
        _emit(rl(0)[:4 * KS - 4])
        cp_w0[1].wait()
        _emit(rl(0)[4 * KS - 4:4 * KS] + pp(0, 6, (0, 1), k1=KS))
        cp_w0[2].wait()
        cp_x0[1].wait()
        ln1 = layernorm(0, 32, 2, (0, 1, 2, 4), PIN + zero)
        _emit(pp(6, 8, (0, 1), k1=KS), _merge(rl(zero)[4 * KS:], ln1[:3]), 1)
        _emit(pp(0, 8, (0, 1), k0=KS), ln1[3:], 4)
        _emit(pp(0, 4, (2, 3)))
        cp_w[1].wait()
        _emit(pp(4, 8, (2, 3)), rl(1 + zero))
        _emit(pp(8, 14))
        cp_w[2].wait()
        cp_w[3].wait()
        _emit(pp(14, 16), rl(2 + zero))
        _emit(pp(16, 24), rl(3 + zero), 2)

        def pre_body(it, carry):
            w_wait(2 * it + 4)
            w_wait(2 * it + 5)
            x_copy(it + 1).wait()

            @pl.when(it > 0)
            def _():
                w_wait(it + 9)

            scores[:] = carry
            for half in range(2):
                ln = layernorm(it + 1, 32 * half, 1, (0, 1, 3, 5), PIN)
                rls = _merge(rl(4 + half + 2 * jnp.minimum(it, 2)),
                             rl(jnp.where(it > 0, it + 9, 0))[10 * half:10 * half + 10])
                _emit(pp(24 + 8 * half, 32 + 8 * half, dc=2 * it), _merge(rls, ln), 2)
            return tuple(scores)

        scores[:] = lax.fori_loop(0, 3, pre_body, tuple(scores))
        for cp in cp_ffn:
            cp.wait()
        _emit(pp(72, 75), [top_c], 1)
        _emit(pp(75, 3 * H - NF) + [P(vfill, 0, i) for i in range(NF)],
              [P(fn, n) for n in range(14) for fn in (ffn_gate, ffn_up)]
              + [P(ffn_down, n, k0) for k0 in range(0, 14, FKC) for n in range(KT)]
              + [ffn_scatter], 9)
        for cp in cp_wo + [cp_m0]:
            cp.wait()

        def finish(s, lo, n, s_val):
            b = xb32[s, lo // 8:(lo + n) // 8].reshape(n, D)
            x = xbuf[s, lo // 8:(lo + n) // 8, :, 0:D].astype(f32).reshape(n, D)
            hb = 0.5 * b
            g = hb * jnp.tanh(hb) + hb
            obuf[s, lo // 8:(lo + n) // 8] = (x + s_val * g).reshape(n // 8, 8, D).astype(bf16)

        col = lax.broadcasted_iota(jnp.int32, (8, 80), 1)
        row = lax.broadcasted_iota(jnp.int32, (8, 80), 0)
        is_h0 = (col < 32) | ((col >= 64) & (col < 72))
        own = (is_h0, jnp.logical_not(is_h0))
        cj = col & 31
        cpos = jnp.where(col < 64, jnp.where(cj < 8, cj, cj + 8), 8 + (col & 7))
        groups = ((0, 4), (1, 5), (2, 6), (3, 7), (8, 9))
        causal = [None] + [cpos <= row + 8 + 8 * i for i in (1, 2, 3)] + [cpos <= row + 8]
        scale = E ** -0.5

        def step(g, j, mem, vcur, held, fillers):
            s = 4 * g + j
            rows_b = pl.ds(pl.multiple_of(32 * g, 32) + 8 * j, 8)
            xa = [jnp.concatenate([act[XA0 + KT * jj + k, rows_b, :] for k in range(KT)], axis=1)
                  for jj in (1, 2, 3)]
            lhs = jnp.concatenate([mem] + xa, axis=0).astype(bf16)
            nrow = 48 if j % 2 else 32
            order, pqk, ppv, dv, dpv, split, pop = STEPS[j]
            st = {}

            def brows(h):
                if h >= 3 * H - NF:
                    return vcur[h - (3 * H - NF)][8 * j:8 * j + 8]
                return act[h, rows_b, :]

            def proj(t, hp, par):
                if not 0 <= hp < NP:
                    return
                h = t * H + 2 * hp
                st['y', par] = jnp.dot(lhs, wtile(h + par), preferred_element_type=f32)
                if par == 1:
                    st['qkv', t, hp] = jnp.concatenate(
                        [st['y', 0], st['y', 1], brows(h), brows(h + 1)], axis=0).astype(bf16)

            def qk(hp):
                sc = lax.dot_general(st['qkv', 0, hp], st['qkv', 1, hp], NT,
                                     preferred_element_type=f32)
                rows = [None] * 10
                for gs, cm in zip(groups, causal):
                    for r, hm in zip(gs, own):
                        sg = sc[8 * r:8 * r + 8] * scale
                        if cm is not None:
                            sg = jnp.where(cm, sg, -1000000000.0)
                        sg = jnp.where(hm, sg, -jnp.inf)
                        e = jnp.exp(sg - jnp.max(sg, axis=-1, keepdims=True))
                        l = jnp.sum(e, axis=-1, keepdims=True)
                        rows[r] = e * pl.reciprocal(l, approx=True)
                st['p', hp] = jnp.concatenate(rows, axis=0).astype(bf16)

            def pv(hp):
                o = jnp.dot(st['p', hp], st['qkv', 2, hp], preferred_element_type=f32)
                for par in (0, 1):
                    h = 2 * hp + par
                    oa, ob = o[32 * par:32 * par + 32], o[64 + 8 * par:72 + 8 * par]
                    if j % 2:
                        oa = jnp.concatenate([oa, held[h], ob], axis=0)
                    else:
                        held[h] = ob
                    st['o', h] = oa

            def oproj(n, h0, h1):
                a = jnp.concatenate([st['o', h] for h in range(h0, h1)], axis=1).astype(bf16)
                return jnp.dot(a, wo[n, h0 * 128:h1 * 128, :], preferred_element_type=f32)

            for u in fillers:
                u()
            for t in range(NP + KT):
                for i in range(7):
                    if pqk == i and 0 <= t - 1 < NP:
                        qk(t - 1)
                    if ppv == i and 0 <= t - dpv < NP:
                        pv(t - dpv)
                    if i < 6:
                        which = 'qkv'.index(order[i // 2])
                        proj(which, t - dv if which == 2 else t, i % 2)
                        if t >= NP and i == pop:
                            accs[t - NP, 0:nrow] = oproj(t - NP, 0, split)
            acc = jnp.concatenate([accs[n, 0:nrow] + oproj(n, split, H) for n in range(KT)], axis=1)
            finish(s, 8, 24, acc[8:32])
            if j % 2:
                finish(s - 1, 0, 8, acc[32:40])
                finish(s, 0, 8, acc[40:48])
            return _rb(acc[0:8])

        def group(g, mem):
            vcur = [vnext[i] for i in range(NF)]
            gn = jnp.minimum(g + 1, NG - 1)
            held = {}
            for j in range(4):
                fillers = [P(vfill, gn, i) for i in range(NF) if FILL[i] == j]
                mem = step(g, j, mem, vcur, held, fillers)
                if j == 2:
                    out_copy(2 * g).start()
            out_copy(2 * g + 1).start()
            return mem

        lax.fori_loop(0, NG, group, mem0_ref[0:8, :].astype(f32))
        return carry

    lax.fori_loop(0, zero + 1, everything, 0)
    for g in range(2 * NG):
        out_copy(g).wait()


@functools.partial(jax.jit, static_argnames=("A_seg_len",))
def pallas_recurrent_scan__memory_aug_recurrent_mem_tr__moe_arch_mod__prompt_kernel(
    A_x: jax.Array,
    A_mem0: jax.Array,
    A_Wq: jax.Array,
    A_Wk: jax.Array,
    A_Wv: jax.Array,
    A_Wo: jax.Array,
    A_seg_len,
    B_x: jax.Array,
    B_w_r: jax.Array,
    B_w_gate: jax.Array,
    B_w_up: jax.Array,
    B_w_down: jax.Array,
):
    del B_x
    assert A_seg_len == SEG
    assert A_x.shape == (1, S, D) and A_Wq.shape == (D, H, E) and B_w_gate.shape == (D, F)
    hbm = pl.BlockSpec(memory_space=pl.ANY)
    out = pl.pallas_call(
        _kernel,
        out_shape=jax.ShapeDtypeStruct((NSEG, 4, 8, D), bf16),
        in_specs=[hbm] * 10,
        out_specs=hbm,
        scratch_shapes=[
            pltpu.VMEM((NSEG, 4, 8, 1024), bf16),
            pltpu.VMEM((NSEG, 4, 8, D), f32),
            pltpu.VMEM((NSEG * 4, D), u32),
            pltpu.VMEM((32, D), f32),
            pltpu.VMEM((16, F), f32),
            pltpu.VMEM((NCH, D, 8, E), bf16),
            pltpu.VMEM((KT, H * E, 128), bf16),
            pltpu.VMEM((PIN + 1, NSEG * 8, E), f32),
            pltpu.VMEM((NF, 32, E), f32),
            pltpu.VMEM((F, D), bf16),
            pltpu.VMEM((F, D), bf16),
            pltpu.VMEM((F, D), bf16),
            pltpu.VMEM((NSEG, 4, 8, D), bf16),
            pltpu.VMEM((KT, 64, 128), f32),
            pltpu.VMEM((64, D), bf16),
            pltpu.SemaphoreType.DMA((29,)),
            pltpu.SemaphoreType.DMA((2 * NG,)),
            pltpu.VMEM((NCH, 2, 4 * PITCH, E), u32),
            pltpu.VMEM((D,), bf16),
        ],
        compiler_params=pltpu.CompilerParams(
            vmem_limit_bytes=120 * 1024 * 1024,
            disable_bounds_checks=True, disable_semaphore_checks=True),
    )(A_x.reshape(NSEG, 4, 8, D), A_mem0.reshape(M, D), A_Wq, A_Wk, A_Wv, A_Wo.reshape(H * E, D),
      B_w_r, B_w_gate.T, B_w_up.T, B_w_down)
    return out.reshape(1, S, D)
```

```python
import functools

import jax
import jax.numpy as jnp
from jax import lax
import jax.experimental.pallas as pl
import jax.experimental.pallas.tpu as pltpu

bf16 = jnp.bfloat16
f32 = jnp.float32
u32 = jnp.uint32
P = functools.partial

S, D, H, E = 2048, 640, 32, 128
M, SEG = 8, 32
NSEG = S // SEG
NG = NSEG // 4
NP = H // 2
F, C = 1728, 8
KT = D // 128
NCH = 12
PITCH = 328
XA0 = 3 * H
PIN = XA0 + 4 * KT
EPS_BF16 = 1.0013580322265625e-05
KEY0 = 0x3F800000
NT = (((1,), (1,)), ((), ()))

STEPS = (('kqv', 3, 4, 2, 3, 22, 0),
         ('kqv', 6, 5, 2, 3, 26, 2),
         ('qkv', 5, 5, 1, 3, 24, 2),
         ('kqv', 4, 3, 1, 3, 22, 0))
FILL = (1, 1, 2, 2, 3, 3)
NF = len(FILL)
FKC = 5


def _rb(v):
    return v.astype(bf16).astype(f32)


def _merge(a, b):
    keyed = [((i + 0.5) / len(a), 0, t) for i, t in enumerate(a)]
    keyed += [((i + 0.5) / len(b), 1, t) for i, t in enumerate(b)]
    return [t for _, _, t in sorted(keyed, key=lambda e: e[:2])]


def _emit(units, side=(), early=0):
    done = 0
    for i, unit in enumerate(units):
        unit()
        want = min(len(side), (len(side) * (i + 1)) // (len(units) - early))
        for task in side[done:want]:
            task()
        done = want


def _kernel(x_hbm, mem0_hbm, wq_hbm, wk_hbm, wv_hbm, wo_hbm, wr_hbm, wg_hbm, wu_hbm, wd_hbm,
            out_hbm,
            xbuf, xb32, xnb, sel_ref, hh_ref, wraw, wo, act, vnext,
            wg, wu, wd, obuf, accs, mem0_ref, sems, osems, wqkv, wr_ref):
    w_hbm = (wq_hbm, wk_hbm, wv_hbm)

    def x_copy(j):
        return pltpu.make_async_copy(x_hbm.at[:, j], xbuf.at[:, j, :, pl.ds(0, D)],
                                     sems.at[25 + j])

    def w_copy(c, src):
        return pltpu.make_async_copy(src, wraw.at[c], sems.at[1 + c])

    def w_wait(c):
        w_copy(c, wq_hbm.at[:, pl.ds(0, 8), :]).wait()

    cp_x = [None] + [x_copy(j) for j in range(1, 4)]
    cp_w = [None] + [w_copy(c, w_hbm[c // 4].at[:, pl.ds(8 * (c % 4), 8), :])
                     for c in range(1, NCH)]
    cp_w0 = [pltpu.make_async_copy(wq_hbm.at[pl.ds(lo, hi - lo), pl.ds(0, 8), :],
                                   wraw.at[0, pl.ds(lo, hi - lo)], sems.at[sem])
             for sem, lo, hi in ((13, 0, 128), (14, 128, 384), (0, 384, D))]
    cp_x0 = [pltpu.make_async_copy(x_hbm.at[pl.ds(32 * i, 32), 0],
                                   xbuf.at[pl.ds(32 * i, 32), 0, :, pl.ds(0, D)], sems.at[sem])
             for i, sem in enumerate((25, 1))]
    cp_ffn = [pltpu.make_async_copy(src, dst, sems.at[15 + i])
              for i, (src, dst) in enumerate(((wg_hbm, wg), (wu_hbm, wu), (wd_hbm, wd)))]
    cp_wo = [pltpu.make_async_copy(wo_hbm.at[:, pl.ds(128 * n, 128)], wo.at[n], sems.at[18 + n])
             for n in range(KT)]
    cp_wr = pltpu.make_async_copy(wr_hbm, wr_ref, sems.at[23])
    cp_m0 = pltpu.make_async_copy(mem0_hbm, mem0_ref.at[pl.ds(0, 8)], sems.at[24])
    for cp in ([cp_wr, cp_x0[0]] + cp_w0 + [cp_x0[1]] + cp_w[1:6] + [cp_x[1]] + cp_w[6:8]
               + [cp_x[2], cp_w[10]] + cp_w[8:10] + [cp_x[3], cp_w[11]] + cp_ffn + cp_wo
               + [cp_m0]):
        cp.start()
    zero = lax.fori_loop(0, 2, lambda i, c: (c + i) >> 1, 0)

    def out_copy(g):
        segs = pl.ds(g * 2, 2)
        return pltpu.make_async_copy(obuf.at[segs], out_hbm.at[segs], osems.at[g])

    def everything(_, carry):
        cp_x0[0].wait()
        cp_wr.wait()

        wr = wr_ref[...].astype(f32).reshape(1, D)
        lane = lax.broadcasted_iota(jnp.int32, (8, 128), 1)
        scores = [jnp.zeros((8, 128), f32), jnp.zeros((8, 128), f32)]

        def layernorm(j, s0, nb, lag, pin):
            st = {}
            n = 32 // nb
            lane_j = lane - j

            def load(i):
                return xbuf[pl.ds(s0 + nb * i, nb), j, :, 0:D].astype(f32).reshape(8 * nb, D)

            def mean(i):
                st['mu', i] = jnp.mean(load(i), axis=-1, keepdims=True)

            def var(i):
                xc = load(i) - st['mu', i]
                st['var', i] = jnp.mean(xc * xc, axis=-1, keepdims=True)

            def norm(i):
                lo, hi = s0 + nb * i, s0 + nb * (i + 1)
                v = _rb(_rb(st['var', i]) + EPS_BF16)
                den = _rb(v * lax.rsqrt(v))
                inv = pl.reciprocal(den, approx=True)
                inv = inv * (2.0 - den * inv)
                xn = (load(i) - _rb(st['mu', i])) * inv
                if len(lag) == 3:
                    xnb[4 * lo:4 * hi, :] = pltpu.bitcast(xn.astype(bf16), u32)
                    if pin is not None:
                        act[pin, 0:8, :] = xn[0:8, 0:128]
                    return
                xb32[pl.ds(lo, nb), j] = xn.reshape(nb, 8, D)
                for k in range(KT):
                    act[XA0 + KT * j + k, 8 * lo:8 * hi, :] = xn[:, 128 * k:128 * (k + 1)]
                st['r', i] = jnp.sum(xn * wr, axis=-1, keepdims=True)

            def score(i):
                v = s0 // 32
                for k in range(nb):
                    scores[v] = jnp.where(lane_j == 4 * (nb * i + k), st['r', i][8 * k:8 * k + 8],
                                          scores[v])
                act[pin, 0:8, :] = scores[v]

            def stage(t):
                for d, fn in zip(lag, (mean, var, norm, score)):
                    if 0 <= t - d < n:
                        fn(t - d)

            return [P(stage, t) for t in range(n + lag[-1])]

        def late_b(s0):
            st = {}

            def stage(t):
                if t < 16:
                    lo = s0 + 2 * t
                    xn = pltpu.bitcast(xnb[4 * lo:4 * lo + 8, :], bf16).astype(f32)
                    xb32[lo:lo + 2, 0] = xn.reshape(2, 8, D)
                    st[t] = jnp.sum(xn * wr, axis=-1, keepdims=True)
                if t >= 2:
                    v = s0 // 32
                    for k in range(2):
                        scores[v] = jnp.where(lane == 4 * (2 * (t - 2) + k),
                                              st[t - 2][8 * k:8 * k + 8], scores[v])
                    act[PIN + zero, 0:8, :] = scores[v]

            return [P(stage, t) for t in range(18)]

        def relayout(c, i):
            for dd in range(16 * i, 16 * i + 16):
                a = pltpu.bitcast(wraw[c, 2 * dd], u32)
                b = pltpu.bitcast(wraw[c, 2 * dd + 1], u32)
                rows = pl.ds(dd, 4, stride=PITCH)
                wqkv[c, 0, rows, :] = (a & jnp.uint32(0xFFFF)) | (b << 16)
                wqkv[c, 1, rows, :] = (a >> 16) | (b & jnp.uint32(0xFFFF0000))

        def wtile(h, dc=0, k0=0, k1=KT):
            start = (h // 2 % 4) * PITCH
            w = wqkv[h // 8 + dc, h % 2, start + 64 * k0:start + 64 * k1, :]
            return pltpu.bitcast(w, bf16)

        def prepass(h, mb, dc=0, k0=0, k1=KT):
            rows = slice(128 * mb, 128 * (mb + 1))
            lhs = pltpu.bitcast(xnb[64 * mb:64 * (mb + 1), 128 * k0:128 * k1], bf16)
            y = jnp.dot(lhs, wtile(h, dc, k0, k1), preferred_element_type=f32)
            act[h + 8 * dc, rows, :] = y if k0 == 0 else act[h + 8 * dc, rows, :] + y

        def vfill(g, i):
            r0 = g * 16 if isinstance(g, int) else pl.multiple_of(g * 16, 16)
            lhs = pltpu.bitcast(xnb[pl.ds(r0, 16), :], bf16)
            vnext[i] = jnp.dot(lhs, wtile(3 * H - NF + i), preferred_element_type=f32)

        def pp(h0, h1, mbs=range(4), **kw):
            return [P(prepass, h, mb, **kw) for h in range(h0, h1) for mb in mbs]

        def rl(c):
            return [P(relayout, c, i) for i in range(20)]

        route = {}

        def top_c():
            r = _rb(jnp.concatenate(scores, axis=1))
            tok = (lax.broadcasted_iota(jnp.int32, (8, 256), 1) * 8
                   + lax.broadcasted_iota(jnp.int32, (8, 256), 0))
            bits = lax.shift_right_logical(pltpu.bitcast(r, jnp.int32), 16)
            rank = jnp.where(bits >= 0x8000, 0x10000 - bits, bits + 0x8000)
            rank = jnp.where(r == r, rank, 0)
            key = pltpu.bitcast(rank * 2048 + (S - 1 - tok) + KEY0, f32)
            row16 = lax.broadcasted_iota(jnp.int32, (16, 128), 0)
            sel_ref[8:16, :] = jnp.zeros((8, D), f32)
            picked = jnp.full((16, 128), KEY0 + 0x8000 * 2048, jnp.int32)
            idxs = []
            for j in range(C):
                best = jnp.max(key, keepdims=True)
                key = jnp.where(key == best, 0.0, key)
                code = pltpu.bitcast(jnp.broadcast_to(best, (16, 128)), jnp.int32)
                picked = jnp.where(row16 == j, code, picked)
                t = (S - 1) - ((code[0, 0] - KEY0) & (S - 1))
                idx = (jnp.clip(t >> 5, 0, NSEG - 1), jnp.clip((t >> 3) & 3, 0, 3),
                       jnp.clip(t & 7, 0, 7))
                idxs.append(idx)
                sel_ref[j:j + 1, :] = xb32[idx[0], idx[1], pl.ds(idx[2], 1), :]
            rank = lax.shift_right_logical(picked - KEY0, 11)
            bits = jnp.where(rank >= 0x8000, rank - 0x8000, 0x10000 - rank)
            route['idx'] = idxs
            route['gate'] = jax.nn.sigmoid(pltpu.bitcast(bits << 16, f32))

        def ffn_gate(n):
            cols = slice(128 * n, min(128 * (n + 1), F))
            hg = lax.dot_general(sel_ref[0:16, :].astype(bf16), wg[cols, :], NT,
                                 preferred_element_type=f32)
            route['g', n] = hg * jax.nn.sigmoid(hg)

        def ffn_up(n):
            cols = slice(128 * n, min(128 * (n + 1), F))
            hu = lax.dot_general(sel_ref[0:16, :].astype(bf16), wu[cols, :], NT,
                                 preferred_element_type=f32)
            hh_ref[:, cols] = route['g', n] * hu

        def ffn_down(n, k0):
            cols = slice(128 * n, 128 * (n + 1))
            ks = slice(128 * k0, min(128 * (k0 + FKC), F))
            y = jnp.dot(hh_ref[:, ks].astype(bf16), wd[ks, cols], preferred_element_type=f32)
            src = slice(16, 32) if k0 else slice(0, 16)
            sel_ref[16:32, cols] = sel_ref[src, cols] + y * route['gate']

        def ffn_scatter():
            for j in range(C):
                idx = route['idx'][j]
                xb32[idx[0], idx[1], pl.ds(idx[2], 1), :] = sel_ref[16 + j:17 + j, :]

        _emit(layernorm(0, 0, 8, (0, 1, 2), None))
        cp_w0[0].wait()
        _emit(rl(0)[:4] + pp(0, 8, (0, 1), k1=1))
        cp_w0[1].wait()
        _emit(rl(0)[4:12] + pp(0, 8, (0, 1), k0=1, k1=3))
        cp_w0[2].wait()
        cp_x0[1].wait()
        ln1 = layernorm(0, 32, 4, (0, 1, 2), PIN + zero)
        _emit(rl(0)[12:] + ln1[:2])
        _emit(pp(0, 8, (0, 1), k0=3), ln1[2:], 4)
        _emit(pp(0, 4, (2, 3)))
        cp_w[1].wait()
        _emit(pp(4, 8, (2, 3)), rl(1 + zero))
        _emit(pp(8, 14), late_b(0) + late_b(32), 1)
        cp_w[2].wait()
        cp_w[3].wait()
        _emit(pp(14, 16), rl(2 + zero))
        _emit(pp(16, 24), rl(3 + zero), 2)

        def pre_body(it, carry):
            w_wait(2 * it + 4)
            w_wait(2 * it + 5)
            x_copy(it + 1).wait()

            @pl.when(it > 0)
            def _():
                w_wait(it + 9)

            scores[:] = carry
            for half in range(2):
                ln = layernorm(it + 1, 32 * half, 1, (0, 1, 3, 5), PIN)
                rls = _merge(rl(4 + half + 2 * jnp.minimum(it, 2)),
                             rl(jnp.where(it > 0, it + 9, 0))[10 * half:10 * half + 10])
                _emit(pp(24 + 8 * half, 32 + 8 * half, dc=2 * it), _merge(rls, ln), 2)
            return tuple(scores)

        scores[:] = lax.fori_loop(0, 3, pre_body, tuple(scores))
        for cp in cp_ffn:
            cp.wait()
        _emit(pp(72, 75), [top_c], 1)
        _emit(pp(75, 3 * H - NF) + [P(vfill, 0, i) for i in range(NF)],
              [P(fn, n) for n in range(14) for fn in (ffn_gate, ffn_up)]
              + [P(ffn_down, n, k0) for k0 in range(0, 14, FKC) for n in range(KT)]
              + [ffn_scatter], 9)
        for cp in cp_wo + [cp_m0]:
            cp.wait()

        def finish(s, lo, n, s_val):
            b = xb32[s, lo // 8:(lo + n) // 8].reshape(n, D)
            x = xbuf[s, lo // 8:(lo + n) // 8, :, 0:D].astype(f32).reshape(n, D)
            hb = 0.5 * b
            g = hb * jnp.tanh(hb) + hb
            obuf[s, lo // 8:(lo + n) // 8] = (x + s_val * g).reshape(n // 8, 8, D).astype(bf16)

        col = lax.broadcasted_iota(jnp.int32, (8, 80), 1)
        row = lax.broadcasted_iota(jnp.int32, (8, 80), 0)
        is_h0 = (col < 32) | ((col >= 64) & (col < 72))
        own = (is_h0, jnp.logical_not(is_h0))
        cj = col & 31
        cpos = jnp.where(col < 64, jnp.where(cj < 8, cj, cj + 8), 8 + (col & 7))
        groups = ((0, 4), (1, 5), (2, 6), (3, 7), (8, 9))
        causal = [None] + [cpos <= row + 8 + 8 * i for i in (1, 2, 3)] + [cpos <= row + 8]
        scale = E ** -0.5

        def step(g, j, mem, vcur, held, fillers):
            s = 4 * g + j
            rows_b = pl.ds(pl.multiple_of(32 * g, 32) + 8 * j, 8)
            xa = [jnp.concatenate([act[XA0 + KT * jj + k, rows_b, :] for k in range(KT)], axis=1)
                  for jj in (1, 2, 3)]
            lhs = jnp.concatenate([mem] + xa, axis=0).astype(bf16)
            nrow = 48 if j % 2 else 32
            order, pqk, ppv, dv, dpv, split, pop = STEPS[j]
            st = {}

            def brows(h):
                if h >= 3 * H - NF:
                    return vcur[h - (3 * H - NF)][8 * j:8 * j + 8]
                return act[h, rows_b, :]

            def proj(t, hp, par):
                if not 0 <= hp < NP:
                    return
                h = t * H + 2 * hp
                st['y', par] = jnp.dot(lhs, wtile(h + par), preferred_element_type=f32)
                if par == 1:
                    st['qkv', t, hp] = jnp.concatenate(
                        [st['y', 0], st['y', 1], brows(h), brows(h + 1)], axis=0).astype(bf16)

            def qk(hp):
                sc = lax.dot_general(st['qkv', 0, hp], st['qkv', 1, hp], NT,
                                     preferred_element_type=f32)
                rows = [None] * 10
                for gs, cm in zip(groups, causal):
                    for r, hm in zip(gs, own):
                        sg = sc[8 * r:8 * r + 8] * scale
                        if cm is not None:
                            sg = jnp.where(cm, sg, -1000000000.0)
                        sg = jnp.where(hm, sg, -jnp.inf)
                        e = jnp.exp(sg - jnp.max(sg, axis=-1, keepdims=True))
                        l = jnp.sum(e, axis=-1, keepdims=True)
                        rows[r] = e * pl.reciprocal(l, approx=True)
                st['p', hp] = jnp.concatenate(rows, axis=0).astype(bf16)

            def pv(hp):
                o = jnp.dot(st['p', hp], st['qkv', 2, hp], preferred_element_type=f32)
                for par in (0, 1):
                    h = 2 * hp + par
                    oa, ob = o[32 * par:32 * par + 32], o[64 + 8 * par:72 + 8 * par]
                    if j % 2:
                        oa = jnp.concatenate([oa, held[h], ob], axis=0)
                    else:
                        held[h] = ob
                    st['o', h] = oa

            def oproj(n, h0, h1):
                a = jnp.concatenate([st['o', h] for h in range(h0, h1)], axis=1).astype(bf16)
                return jnp.dot(a, wo[n, h0 * 128:h1 * 128, :], preferred_element_type=f32)

            for u in fillers:
                u()
            for t in range(NP + KT):
                for i in range(7):
                    if pqk == i and 0 <= t - 1 < NP:
                        qk(t - 1)
                    if ppv == i and 0 <= t - dpv < NP:
                        pv(t - dpv)
                    if i < 6:
                        which = 'qkv'.index(order[i // 2])
                        proj(which, t - dv if which == 2 else t, i % 2)
                        if t >= NP and i == pop:
                            accs[t - NP, 0:nrow] = oproj(t - NP, 0, split)
            acc = jnp.concatenate([accs[n, 0:nrow] + oproj(n, split, H) for n in range(KT)], axis=1)
            finish(s, 8, 24, acc[8:32])
            if j % 2:
                finish(s - 1, 0, 8, acc[32:40])
                finish(s, 0, 8, acc[40:48])
            return _rb(acc[0:8])

        def group(g, mem):
            vcur = [vnext[i] for i in range(NF)]
            gn = jnp.minimum(g + 1, NG - 1)
            held = {}
            for j in range(4):
                fillers = [P(vfill, gn, i) for i in range(NF) if FILL[i] == j]
                mem = step(g, j, mem, vcur, held, fillers)
                if j == 2:
                    out_copy(2 * g).start()
            out_copy(2 * g + 1).start()
            return mem

        lax.fori_loop(0, NG, group, mem0_ref[0:8, :].astype(f32))
        return carry

    lax.fori_loop(0, zero + 1, everything, 0)
    for g in range(2 * NG):
        out_copy(g).wait()


@jax.jit
def pallas_recurrent_scan__memory_aug_recurrent_mem_tr__moe_arch_mod__prompt_kernel(
    A_x: jax.Array,
    A_mem0: jax.Array,
    A_Wq: jax.Array,
    A_Wk: jax.Array,
    A_Wv: jax.Array,
    A_Wo: jax.Array,
    A_seg_len: jax.Array,
    B_x: jax.Array,
    B_w_r: jax.Array,
    B_w_gate: jax.Array,
    B_w_up: jax.Array,
    B_w_down: jax.Array,
):
    del B_x
    del A_seg_len
    assert A_x.shape == (1, S, D) and A_Wq.shape == (D, H, E) and B_w_gate.shape == (D, F)
    hbm = pl.BlockSpec(memory_space=pl.ANY)
    out = pl.pallas_call(
        _kernel,
        out_shape=jax.ShapeDtypeStruct((NSEG, 4, 8, D), bf16),
        in_specs=[hbm] * 10,
        out_specs=hbm,
        scratch_shapes=[
            pltpu.VMEM((NSEG, 4, 8, 1024), bf16),
            pltpu.VMEM((NSEG, 4, 8, D), f32),
            pltpu.VMEM((NSEG * 4, D), u32),
            pltpu.VMEM((32, D), f32),
            pltpu.VMEM((16, F), f32),
            pltpu.VMEM((NCH, D, 8, E), bf16),
            pltpu.VMEM((KT, H * E, 128), bf16),
            pltpu.VMEM((PIN + 1, NSEG * 8, E), f32),
            pltpu.VMEM((NF, 32, E), f32),
            pltpu.VMEM((F, D), bf16),
            pltpu.VMEM((F, D), bf16),
            pltpu.VMEM((F, D), bf16),
            pltpu.VMEM((NSEG, 4, 8, D), bf16),
            pltpu.VMEM((KT, 64, 128), f32),
            pltpu.VMEM((64, D), bf16),
            pltpu.SemaphoreType.DMA((29,)),
            pltpu.SemaphoreType.DMA((2 * NG,)),
            pltpu.VMEM((NCH, 2, 4 * PITCH, E), u32),
            pltpu.VMEM((D,), bf16),
        ],
        compiler_params=pltpu.CompilerParams(
            vmem_limit_bytes=120 * 1024 * 1024,
            disable_bounds_checks=True, disable_semaphore_checks=True),
    )(A_x.reshape(NSEG, 4, 8, D), A_mem0.reshape(M, D), A_Wq, A_Wk, A_Wv, A_Wo.reshape(H * E, D),
      B_w_r, B_w_gate.T, B_w_up.T, B_w_down)
    return out.reshape(1, S, D)
```
